```python
import jax
import jax.numpy as jnp

def _softmax(x, axis=-1):
    return jax.nn.softmax(x, axis=axis)

def _gelu(x):
    return jax.nn.gelu(x, approximate=True)

def _silu(x):
    return jax.nn.silu(x)

def _sigmoid(x):
    return jax.nn.sigmoid(x)

def _layernorm(x, axis=-1, eps=1e-05):
    m = jnp.mean(x, axis=axis, keepdims=True)
    v = jnp.var(x, axis=axis, keepdims=True)
    return (x - m) / jnp.sqrt(v + eps)

def _scatter_add(tgt, idx, src, axis=0):
    return tgt.at[idx].add(src)

def _segment_sum(src, seg, n):
    return jax.ops.segment_sum(src, seg, n)

class _Rng:

    def __init__(self, key):
        self._k = key

    def _next(self):
        self._k, sub = jax.random.split(self._k)
        return sub

    def normal(self, shape):
        return jax.random.normal(self._next(), shape, dtype=jnp.bfloat16)

    def randint(self, lo, hi, shape):
        return jax.random.randint(self._next(), shape, lo, hi, dtype=jnp.int32)

    def uniform(self, shape, lo=0.0, hi=1.0):
        return jax.random.uniform(self._next(), shape, jnp.bfloat16, lo, hi)

    def permutation(self, n):
        return jax.random.permutation(self._next(), n)
kernel_name = 'gated_mix__memory_aug_recurrent_mem_tr__sliding_local_dilated__prompt'

def setup_inputs():
    _rng = _Rng(jax.random.key(int.from_bytes(__import__("os").urandom(4), "little")))
    _w = lambda a: (lambda t: t.astype(jnp.bfloat16) if jnp.issubdtype(t.dtype, jnp.floating) else t)(jnp.asarray(a))

    def _A_setup():
        B, S, Dm = (1, 2048, 640)
        H, Dh = (32, 192)
        M, seg = (8, 32)
        seg = min(seg, S)
        S = S // seg * seg
        return {'x': _w((lambda *s: _rng.normal(s) * 0.05)(B, S, Dm)), 'mem0': _w((lambda *s: _rng.normal(s) * 0.05)(B, M, Dm)), 'Wq': _w((lambda *s: _rng.normal(s) * 0.05)(Dm, H, Dh) * Dm ** (-0.5)), 'Wk': _w((lambda *s: _rng.normal(s) * 0.05)(Dm, H, Dh) * Dm ** (-0.5)), 'Wv': _w((lambda *s: _rng.normal(s) * 0.05)(Dm, H, Dh) * Dm ** (-0.5)), 'Wo': _w((lambda *s: _rng.normal(s) * 0.05)(H, Dh, Dm) * (H * Dh) ** (-0.5)), 'seg_len': seg}
    _A_in = _A_setup()

    def _B_setup():
        B, S, D = (1, 2048, 640)
        return {'x': _w((lambda *s: _rng.normal(s) * 0.05)(B, S, D)), 'wqkv': _w((lambda *s: _rng.normal(s) * 0.05)(D, 3 * D)), 'wo': _w((lambda *s: _rng.normal(s) * 0.05)(D, D))}
    _B_in = _B_setup()
    return {'A_x': _A_in['x'], 'A_mem0': _A_in['mem0'], 'A_Wq': _A_in['Wq'], 'A_Wk': _A_in['Wk'], 'A_Wv': _A_in['Wv'], 'A_Wo': _A_in['Wo'], 'A_seg_len': _A_in['seg_len'], 'B_x': _B_in['x'], 'B_wqkv': _B_in['wqkv'], 'B_wo': _B_in['wo'], 'gate_w': _w((lambda *s: _rng.normal(s) * 0.05)(640))}

def reference(A_x, A_mem0, A_Wq, A_Wk, A_Wv, A_Wo, A_seg_len, B_x, B_wqkv, B_wo, gate_w):

    def _A_ref(x, mem0, Wq, Wk, Wv, Wo, seg_len):
        B, S, Dm = x.shape
        H, Dh = (Wq.shape[1], Wq.shape[2])
        M = mem0.shape[1]
        scale = Dh ** (-0.5)
        n_seg = S // seg_len
        L = M + seg_len
        idx = jnp.arange(L)
        mask = (idx[:, None] < M) | (idx[:, None] >= idx[None, :])
        mem = mem0
        outs = []
        for s in range(n_seg):
            xs = x[:, s * seg_len:(s + 1) * seg_len, :].copy()
            h = jnp.concatenate([mem, xs], axis=1)
            q = jnp.einsum('btd,dhe->bhte', h, Wq)
            k = jnp.einsum('btd,dhe->bhte', h, Wk)
            v = jnp.einsum('btd,dhe->bhte', h, Wv)
            scores = jnp.einsum('bhqe,bhke->bhqk', q, k) * scale
            scores = jnp.where(mask[None, None], scores, -1000000000.0)
            p = _softmax(scores, axis=-1)
            o = jnp.einsum('bhqk,bhke->bhqe', p, v)
            o = jnp.einsum('bhte,hed->btd', o, Wo)
            mem = o[:, :M, :].copy()
            outs.append(o[:, M:, :])
        return jnp.concatenate(outs, axis=1)

    def _B_ref(x, wqkv, wo):
        B, S, D = x.shape
        H = 32
        Dh = D // H
        W, dil = (8, 2)
        qkv = (lambda x, *d: x.transpose(*d))((x @ wqkv).reshape(B, S, 3, H, Dh), 2, 0, 3, 1, 4)
        q, k, v = (qkv[0], qkv[1], qkv[2])
        scale = Dh ** (-0.5)
        pos = jnp.arange(S)
        off = jnp.arange(W) * dil
        idx = pos[:, None] - off[None, :]
        mask = idx >= 0
        idx_c = jnp.where(mask, idx, 0).reshape(-1)
        kg = k[:, :, idx_c, :].reshape(B, H, S, W, Dh)
        vg = v[:, :, idx_c, :].reshape(B, H, S, W, Dh)
        logits = jnp.einsum('bhsd,bhswd->bhsw', q, kg) * scale
        logits = jnp.where(mask[None, None, :, :], logits, -1000000000.0)
        attn = _softmax(logits, axis=-1)
        o = jnp.einsum('bhsw,bhswd->bhsd', attn, vg)
        return (lambda x, *d: x.transpose(*d))(o, 0, 2, 1, 3).reshape(B, S, D) @ wo
    x = A_x
    g = _sigmoid((x * gate_w).sum(-1, keepdims=True))
    a = _A_ref(x, A_mem0, A_Wq, A_Wk, A_Wv, A_Wo, A_seg_len)
    b = _B_ref(x, B_wqkv, B_wo)
    return g * a + (1 - g) * b
```

```python
import functools

import jax
import jax.numpy as jnp
import jax.experimental.pallas as pl
import jax.experimental.pallas.tpu as pltpu

F32 = jnp.float32
BF16 = jnp.bfloat16
U32 = jnp.uint32
LANES = 128
NEG = -1000000000.0

B_HEADS, B_WIN, B_DIL = 32, 8, 2
B_PAD = 16
B_BLK = 256
B_SUB = 32


def _nn(a, b):
    return jax.lax.dot_general(a, b, (((1,), (0,)), ((), ())), preferred_element_type=F32)


def _nt(a, b):
    return jax.lax.dot_general(a, b, (((1,), (1,)), ((), ())), preferred_element_type=F32)


def _pack(w):
    return pltpu.bitcast(w, U32)


def _unpack(w):
    return pltpu.bitcast(w, BF16)


def _iota(shape, dim):
    return jax.lax.broadcasted_iota(jnp.int32, shape, dim)


def _kernel(x_hbm, mem0_ref, wq_hbm, wk_hbm, wv_hbm, wo_hbm, bqkv_hbm, bwo_hbm, gate_ref,
            out_hbm,
            x_v, stage, w_v, wo_v, bqkv_raw, bwo_raw, bqkv_v, bwo_v, kb_v, vb_v, ob_v,
            h_v, out_v, sem_in, sem_w, sem_out, *, seg, dh):
    S, D = x_v.shape
    M = mem0_ref.shape[0]
    L = M + seg
    E = stage.shape[1]
    DT = D // LANES
    PT = 2 * dh // LANES
    n_pair = E // (2 * dh)
    n_blk = S // B_BLK
    w_rows = E // n_blk
    w_hbm = (wq_hbm, wk_hbm, wv_hbm, wo_hbm)

    cp_bqkv = pltpu.make_async_copy(bqkv_hbm, bqkv_raw, sem_in.at[0])
    cp_x = pltpu.make_async_copy(x_hbm, x_v, sem_in.at[1])
    cp_bwo = pltpu.make_async_copy(bwo_hbm, bwo_raw, sem_in.at[2])

    def cp_w(m, c):
        rows = pl.ds(c * w_rows, w_rows)
        return pltpu.make_async_copy(w_hbm[m].at[rows], stage.at[m, rows], sem_w.at[m, c])


    cp_bqkv.start()
    cp_x.start()
    cp_bwo.start()
    for c in range(n_blk):
        for m in range(4):
            cp_w(m, c).start()

    db = D // B_HEADS
    src, dst = _iota((D, D), 0), _iota((D, D), 1)
    perm = (src == (dst % B_HEADS) * db + dst // B_HEADS).astype(F32).astype(BF16)
    perm_t = (dst == (src % B_HEADS) * db + src // B_HEADS).astype(F32).astype(BF16)
    cp_bqkv.wait()
    for m in range(3):
        wp = _nn(bqkv_raw[:, m * D:(m + 1) * D], perm).astype(BF16)
        for t in range(DT):
            bqkv_v[m * DT + t] = _pack(wp[:, t * LANES:(t + 1) * LANES])
    cp_bwo.wait()
    wp = _nn(perm_t, bwo_raw[...]).astype(BF16)
    for t in range(DT):
        bwo_v[t] = _pack(wp[:, t * LANES:(t + 1) * LANES])
    cp_x.wait()

    x_top = x_v[0:B_PAD, :]
    for t in range(DT):
        kb_v[t, 0:B_PAD, :] = jnp.zeros((B_PAD, LANES), F32)
        v0 = _nn(x_top, _unpack(bqkv_v[2 * DT + t]))
        vb_v[t, 0:B_PAD, :] = jnp.broadcast_to(v0[0:1, :], (B_PAD, LANES))

    b_scale = db ** -0.5

    def b_block(i, carry):
        base = pl.multiple_of(i * B_BLK, B_BLK)
        xb = x_v[pl.ds(base, B_BLK), :]
        qb = [_nn(xb, _unpack(bqkv_v[t])) for t in range(DT)]
        for t in range(DT):
            kb_v[t, pl.ds(base + B_PAD, B_BLK), :] = _nn(xb, _unpack(bqkv_v[DT + t]))
            vb_v[t, pl.ds(base + B_PAD, B_BLK), :] = _nn(xb, _unpack(bqkv_v[2 * DT + t]))
        for r in range(0, B_BLK, B_SUB):
            pos = base + r + _iota((B_SUB, LANES), 0)
            logits = []
            for w in range(B_WIN):
                rows = pl.ds(base + (B_PAD + r - w * B_DIL), B_SUB)
                acc = qb[0][r:r + B_SUB] * kb_v[0, rows, :]
                for t in range(1, DT):
                    acc = acc + qb[t][r:r + B_SUB] * kb_v[t, rows, :]
                shift = LANES // 2
                while shift >= B_HEADS:
                    acc = acc + pltpu.roll(acc, shift, 1)
                    shift //= 2
                acc = acc * b_scale
                if w:
                    acc = jnp.where(pos >= w * B_DIL, acc, NEG)
                logits.append(acc)
            mx = functools.reduce(jnp.maximum, logits)
            ex = [jnp.exp(l - mx) for l in logits]
            inv = 1.0 / functools.reduce(jnp.add, ex)
            for t in range(DT):
                acc = None
                for w in range(B_WIN):
                    rows = pl.ds(base + (B_PAD + r - w * B_DIL), B_SUB)
                    term = ex[w] * vb_v[t, rows, :]
                    acc = term if acc is None else acc + term
                ob_v[pl.ds(base + r, B_SUB), t * LANES:(t + 1) * LANES] = (acc * inv).astype(BF16)
        for m in range(4):
            cp_w(m, i).wait()
        for t in range(DT):
            wo_v[t, pl.ds(pl.multiple_of(i * (w_rows // 2), w_rows // 2), w_rows // 2), :] = _pack(
                stage[3, pl.ds(pl.multiple_of(i * w_rows, w_rows), w_rows), t * LANES:(t + 1) * LANES])
        for m in range(3):
            for k in range(w_rows // LANES):
                tile = i * (w_rows // LANES) + k
                rows = pl.ds(pl.multiple_of(tile * LANES, LANES), LANES)
                w_v[m, tile] = _pack(stage[m, rows, :].T)
        return carry

    jax.lax.fori_loop(0, n_blk, b_block, 0)

    h_v[0:M, :] = mem0_ref[...].astype(F32)
    gate = gate_ref[...].astype(F32)
    a_scale = dh ** -0.5
    split = dh - LANES

    def step(s, carry):
        base = pl.multiple_of(s * seg, seg)
        xs = x_v[pl.ds(base, seg), :].astype(F32)
        h_v[M:L, :] = xs

        lo = _iota((L, LANES), 1) < split
        zero = jnp.zeros((L, LANES), F32)
        row, col = _iota((L, 2 * L), 0), _iota((L, 2 * L), 1)
        even = col < L
        visible = (row < M) | (row >= jnp.where(even, col, col - L))

        def project(m, j):
            return [_nn(h_v[...], _unpack(w_v[m, j * PT + t])) for t in range(PT)]

        def two_heads(y):
            top = jnp.concatenate([y[0], jnp.where(lo, y[1], 0.0), zero], axis=1)
            bot = jnp.concatenate([zero, jnp.where(lo, 0.0, y[1]), y[2]], axis=1)
            return jnp.concatenate([top, bot], axis=0).astype(BF16)

        def softmax(sc):
            sc = jnp.where(visible, sc * a_scale, NEG)
            m0 = jnp.max(jnp.where(even, sc, -jnp.inf), axis=1, keepdims=True)
            m1 = jnp.max(jnp.where(even, -jnp.inf, sc), axis=1, keepdims=True)
            e = jnp.exp(sc - jnp.where(even, m0, m1))
            s0 = jnp.sum(jnp.where(even, e, 0.0), axis=1, keepdims=True)
            s1 = jnp.sum(jnp.where(even, 0.0, e), axis=1, keepdims=True)
            return e / jnp.where(even, s0, s1)

        p, o, acc = {}, {}, [None] * DT
        for j in range(n_pair + 3):
            if j < n_pair:
                k = two_heads(project(1, j))
                q = jnp.concatenate(project(0, j), axis=1)
            if 0 <= j - 1 < n_pair:
                v = two_heads(project(2, j - 1))
            if j < n_pair:
                p[j] = softmax(_nt(q, k))
            if 0 <= j - 3 < n_pair:
                oj = o.pop(j - 3)
                for t in range(DT):
                    y = _nn(oj, _unpack(wo_v[t, (j - 3) * dh:(j - 2) * dh, :]))
                    acc[t] = y if acc[t] is None else acc[t] + y
            if 0 <= j - 1 < n_pair:
                o[j - 1] = _nn(p.pop(j - 1), v)

        g = jax.nn.sigmoid(jnp.sum(xs * gate, axis=1, keepdims=True))
        ob = ob_v[pl.ds(base, seg), :]
        for t in range(DT):
            lanes = slice(t * LANES, (t + 1) * LANES)
            h_v[0:M, lanes] = acc[t][0:M]
            b = _nn(ob, _unpack(bwo_v[t]))
            out_v[pl.ds(base, seg), lanes] = (g * acc[t][M:L] + (1.0 - g) * b).astype(out_v.dtype)
        pltpu.make_async_copy(out_v.at[pl.ds(base, seg)], out_hbm.at[pl.ds(base, seg)], sem_out).start()
        return carry

    jax.lax.fori_loop(0, S // seg, step, 0)
    pltpu.make_async_copy(out_v, out_hbm, sem_out).wait()


@functools.partial(jax.jit, static_argnames=("A_seg_len",))
def pallas_gated_mix__memory_aug_recurrent_mem_tr__sliding_local_dilated__prompt_kernel(
    A_x: jax.Array,
    A_mem0: jax.Array,
    A_Wq: jax.Array,
    A_Wk: jax.Array,
    A_Wv: jax.Array,
    A_Wo: jax.Array,
    A_seg_len: int,
    B_x: jax.Array,
    B_wqkv: jax.Array,
    B_wo: jax.Array,
    gate_w: jax.Array,
):
    del B_x
    batch, S, D = A_x.shape
    _, H, dh = A_Wq.shape
    M = A_mem0.shape[1]
    E = H * dh
    seg = int(A_seg_len)
    assert batch == 1 and D % LANES == 0 and 2 * dh == 3 * LANES and H % 2 == 0
    assert S % B_BLK == 0 and S % seg == 0 and E % (S // B_BLK * LANES) == 0

    def w_t(w):
        return jnp.transpose(w, (1, 2, 0)).reshape(E, D)

    hbm = pl.BlockSpec(memory_space=pl.ANY)
    vmem = pl.BlockSpec(memory_space=pltpu.VMEM)
    DT = D // LANES
    out = pl.pallas_call(
        functools.partial(_kernel, seg=seg, dh=dh),
        out_shape=jax.ShapeDtypeStruct((S, D), A_x.dtype),
        in_specs=[hbm, vmem, hbm, hbm, hbm, hbm, hbm, hbm, vmem],
        out_specs=hbm,
        scratch_shapes=[
            pltpu.VMEM((S, D), BF16),
            pltpu.VMEM((4, E, D), BF16),
            pltpu.VMEM((3, E // LANES, D // 2, LANES), U32),
            pltpu.VMEM((DT, E // 2, LANES), U32),
            pltpu.VMEM((D, 3 * D), BF16),
            pltpu.VMEM((D, D), BF16),
            pltpu.VMEM((3 * DT, D // 2, LANES), U32),
            pltpu.VMEM((DT, D // 2, LANES), U32),
            pltpu.VMEM((DT, B_PAD + S, LANES), F32),
            pltpu.VMEM((DT, B_PAD + S, LANES), F32),
            pltpu.VMEM((S, D), BF16),
            pltpu.VMEM((M + seg, D), F32),
            pltpu.VMEM((S, D), A_x.dtype),
            pltpu.SemaphoreType.DMA((3,)),
            pltpu.SemaphoreType.DMA((4, S // B_BLK)),
            pltpu.SemaphoreType.DMA(()),
        ],
        compiler_params=pltpu.CompilerParams(vmem_limit_bytes=110 * 1024 * 1024),
    )(
        A_x.reshape(S, D), A_mem0.reshape(M, D), w_t(A_Wq), w_t(A_Wk), w_t(A_Wv),
        A_Wo.reshape(E, D), B_wqkv, B_wo, gate_w.reshape(1, D),
    )
    return out.reshape(batch, S, D)
```

```python
import functools

import jax
import jax.numpy as jnp
import jax.experimental.pallas as pl
import jax.experimental.pallas.tpu as pltpu

F32 = jnp.float32
BF16 = jnp.bfloat16
U32 = jnp.uint32
LANES = 128
NEG = -1000000000.0

B_HEADS, B_WIN, B_DIL = 32, 8, 2
B_PAD = 16
B_BLK = 256
ORDER = (("K", 0), ("Q", 0), ("P", 2), ("V", 0), ("S", 0), ("O", 4))
B_MM = 64
B_SUB = 32


def _nn(a, b):
    return jax.lax.dot_general(a, b, (((1,), (0,)), ((), ())), preferred_element_type=F32)


def _nt(a, b):
    return jax.lax.dot_general(a, b, (((1,), (1,)), ((), ())), preferred_element_type=F32)


def _pack(w):
    return pltpu.bitcast(w, U32)


def _unpack(w):
    return pltpu.bitcast(w, BF16)


def _iota(shape, dim):
    return jax.lax.broadcasted_iota(jnp.int32, shape, dim)


def _schedule(n_pair, n_tile):
    stages = ORDER
    ops = []
    for j in range(n_pair + max(lag for _, lag in stages)):
        ops += [(op, j - lag) for op, lag in stages if 0 <= j - lag < n_pair]
    return ops + [("B", t) for t in range(n_tile)]


def _kernel(x_hbm, mem0_ref, wq_hbm, wk_hbm, wv_hbm, wo_hbm, bqkv_hbm, bwo_hbm, gate_ref,
            out_hbm,
            x_v, stage, w_v, wo_v, bqkv_raw, bwo_raw, bqkv_v, bwo_v, kb_v, vb_v, ob_v,
            h_v, out_v, sem_in, sem_w, sem_out, *, seg, dh):
    S, D = x_v.shape
    M = mem0_ref.shape[0]
    L = M + seg
    E = stage.shape[1]
    DT = D // LANES
    PT = 2 * dh // LANES
    n_pair = E // (2 * dh)
    n_blk = S // B_BLK
    w_rows = E // n_blk
    w_hbm = (wq_hbm, wk_hbm, wv_hbm, wo_hbm)

    cp_bqkv = pltpu.make_async_copy(bqkv_hbm, bqkv_raw, sem_in.at[0])
    cp_x = pltpu.make_async_copy(x_hbm, x_v, sem_in.at[1])
    cp_bwo = pltpu.make_async_copy(bwo_hbm, bwo_raw, sem_in.at[2])

    def cp_w(m, c):
        rows = pl.ds(c * w_rows, w_rows)
        return pltpu.make_async_copy(w_hbm[m].at[rows], stage.at[m, rows], sem_w.at[m, c])


    def start_w(c):
        for m in range(4):
            cp_w(m, c).start()

    cp_bqkv.start()

    db = D // B_HEADS
    src, dst = _iota((D, D), 0), _iota((D, D), 1)
    perm = (src == (dst % B_HEADS) * db + dst // B_HEADS).astype(F32).astype(BF16)
    perm_t = (dst == (src % B_HEADS) * db + src // B_HEADS).astype(F32).astype(BF16)
    cp_bqkv.wait()
    cp_x.start()
    cp_bwo.start()
    start_w(0)
    for m in range(3):
        wp = _nn(bqkv_raw[:, m * D:(m + 1) * D], perm).astype(BF16)
        for t in range(DT):
            bqkv_v[m * DT + t] = _pack(wp[:, t * LANES:(t + 1) * LANES])
    cp_bwo.wait()
    start_w(1)
    wp = _nn(perm_t, bwo_raw[...]).astype(BF16)
    for t in range(DT):
        bwo_v[t] = _pack(wp[:, t * LANES:(t + 1) * LANES])
    cp_x.wait()

    x_top = x_v[0:B_PAD, :]
    for t in range(DT):
        kb_v[t, 0:B_PAD, :] = jnp.zeros((B_PAD, LANES), F32)
        v0 = _nn(x_top, _unpack(bqkv_v[2 * DT + t]))
        vb_v[t, 0:B_PAD, :] = jnp.broadcast_to(v0[0:1, :], (B_PAD, LANES))

    b_scale = db ** -0.5

    def window_attention(q, base):
        pos = base + _iota((B_SUB, LANES), 0)
        rows = [pl.ds(base + (B_PAD - w * B_DIL), B_SUB) for w in range(B_WIN)]
        logits = []
        for w in range(B_WIN):
            acc = functools.reduce(jnp.add, [q[t] * kb_v[t, rows[w], :] for t in range(DT)])
            shift = LANES // 2
            while shift >= B_HEADS:
                acc = acc + pltpu.roll(acc, shift, 1)
                shift //= 2
            acc = acc * b_scale
            logits.append(jnp.where(pos >= w * B_DIL, acc, NEG) if w else acc)
        mx = functools.reduce(jnp.maximum, logits)
        ex = [jnp.exp(l - mx) for l in logits]
        inv = 1.0 / functools.reduce(jnp.add, ex)
        for t in range(DT):
            acc = functools.reduce(jnp.add, [ex[w] * vb_v[t, rows[w], :] for w in range(B_WIN)])
            ob_v[pl.ds(base, B_SUB), t * LANES:(t + 1) * LANES] = (acc * inv).astype(BF16)

    def b_block(i, carry):
        @pl.when(i + 2 < n_blk)
        def _():
            start_w(i + 2)

        for m in range(4):
            cp_w(m, i).wait()
        for r in range(0, B_BLK, B_MM):
            base = pl.multiple_of(i * B_BLK + r, B_MM)
            xb = x_v[pl.ds(base, B_MM), :]
            for t in range(DT):
                kb_v[t, pl.ds(base + B_PAD, B_MM), :] = _nn(xb, _unpack(bqkv_v[DT + t]))
            qb = [_nn(xb, _unpack(bqkv_v[t])) for t in range(DT)]
            for t in range(DT):
                vb_v[t, pl.ds(base + B_PAD, B_MM), :] = _nn(xb, _unpack(bqkv_v[2 * DT + t]))
            for u in range(0, B_MM, B_SUB):
                window_attention([y[u:u + B_SUB] for y in qb], base + u)
        half = pl.ds(pl.multiple_of(i * (w_rows // 2), w_rows // 2), w_rows // 2)
        for t in range(DT):
            wo_v[t, half, :] = _pack(
                stage[3, pl.ds(pl.multiple_of(i * w_rows, w_rows), w_rows), t * LANES:(t + 1) * LANES])
        for m in range(3):
            for k in range(w_rows // LANES):
                tile = i * (w_rows // LANES) + k
                rows = pl.ds(pl.multiple_of(tile * LANES, LANES), LANES)
                w_v[m, tile] = _pack(stage[m, rows, :].T)
        return carry

    jax.lax.fori_loop(0, n_blk, b_block, 0)

    h_v[0:M, :] = mem0_ref[...].astype(F32)
    gate = gate_ref[...].astype(F32)
    a_scale = dh ** -0.5
    split = dh - LANES

    def step(s, carry):
        base = pl.multiple_of(s * seg, seg)
        xs = x_v[pl.ds(base, seg), :].astype(F32)
        h_v[M:L, :] = xs

        lo = _iota((L, LANES), 1) < split
        zero = jnp.zeros((L, LANES), F32)
        row, col = _iota((L, 2 * L), 0), _iota((L, 2 * L), 1)
        even = col < L
        visible = (row < M) | (row >= jnp.where(even, col, col - L))

        def project(m, j):
            return [_nn(h_v[...], _unpack(w_v[m, j * PT + t])) for t in range(PT)]

        def two_heads(y):
            top = jnp.concatenate([y[0], jnp.where(lo, y[1], 0.0), zero], axis=1)
            bot = jnp.concatenate([zero, jnp.where(lo, 0.0, y[1]), y[2]], axis=1)
            return jnp.concatenate([top, bot], axis=0).astype(BF16)

        def softmax(sc):
            sc = jnp.where(visible, sc * a_scale, NEG)
            m0 = jnp.max(jnp.where(even, sc, -jnp.inf), axis=1, keepdims=True)
            m1 = jnp.max(jnp.where(even, -jnp.inf, sc), axis=1, keepdims=True)
            e = jnp.exp(sc - jnp.where(even, m0, m1))
            s0 = jnp.sum(jnp.where(even, e, 0.0), axis=1, keepdims=True)
            s1 = jnp.sum(jnp.where(even, 0.0, e), axis=1, keepdims=True)
            return e / jnp.where(even, s0, s1)

        ob = ob_v[pl.ds(base, seg), :]
        q, k, v, p, o, b, acc = {}, {}, {}, {}, {}, {}, [None] * DT
        for op, j in _schedule(n_pair, DT):
            if op == "K":
                k[j] = two_heads(project(1, j))
            elif op == "Q":
                q[j] = jnp.concatenate(project(0, j), axis=1)
            elif op == "V":
                v[j] = two_heads(project(2, j))
            elif op == "S":
                p[j] = softmax(_nt(q.pop(j), k.pop(j)))
            elif op == "P":
                o[j] = _nn(p.pop(j), v.pop(j))
            elif op == "O":
                oj = o.pop(j)
                for t in range(DT):
                    y = _nn(oj, _unpack(wo_v[t, j * dh:(j + 1) * dh, :]))
                    acc[t] = y if acc[t] is None else acc[t] + y
            else:
                b[j] = _nn(ob, _unpack(bwo_v[j]))

        g = jax.nn.sigmoid(jnp.sum(xs * gate, axis=1, keepdims=True))
        for t in range(DT):
            lanes = slice(t * LANES, (t + 1) * LANES)
            h_v[0:M, lanes] = acc[t][0:M]
            out_v[pl.ds(base, seg), lanes] = (g * acc[t][M:L] + (1.0 - g) * b[t]).astype(out_v.dtype)
        pltpu.make_async_copy(out_v.at[pl.ds(base, seg)], out_hbm.at[pl.ds(base, seg)], sem_out).start()
        return carry

    jax.lax.fori_loop(0, S // seg, step, 0)
    pltpu.make_async_copy(out_v, out_hbm, sem_out).wait()


@functools.partial(jax.jit, static_argnames=("A_seg_len",))
def pallas_gated_mix__memory_aug_recurrent_mem_tr__sliding_local_dilated__prompt_kernel(
    A_x: jax.Array,
    A_mem0: jax.Array,
    A_Wq: jax.Array,
    A_Wk: jax.Array,
    A_Wv: jax.Array,
    A_Wo: jax.Array,
    A_seg_len: int,
    B_x: jax.Array,
    B_wqkv: jax.Array,
    B_wo: jax.Array,
    gate_w: jax.Array,
):
    del B_x
    batch, S, D = A_x.shape
    _, H, dh = A_Wq.shape
    M = A_mem0.shape[1]
    E = H * dh
    seg = int(A_seg_len)
    assert batch == 1 and D % LANES == 0 and 2 * dh == 3 * LANES and H % 2 == 0
    assert S % B_BLK == 0 and S % seg == 0 and E % (S // B_BLK * LANES) == 0

    def w_t(w):
        return jnp.transpose(w, (1, 2, 0)).reshape(E, D)

    hbm = pl.BlockSpec(memory_space=pl.ANY)
    vmem = pl.BlockSpec(memory_space=pltpu.VMEM)
    DT = D // LANES
    out = pl.pallas_call(
        functools.partial(_kernel, seg=seg, dh=dh),
        out_shape=jax.ShapeDtypeStruct((S, D), A_x.dtype),
        in_specs=[hbm, vmem, hbm, hbm, hbm, hbm, hbm, hbm, vmem],
        out_specs=hbm,
        scratch_shapes=[
            pltpu.VMEM((S, D), BF16),
            pltpu.VMEM((4, E, D), BF16),
            pltpu.VMEM((3, E // LANES, D // 2, LANES), U32),
            pltpu.VMEM((DT, E // 2, LANES), U32),
            pltpu.VMEM((D, 3 * D), BF16),
            pltpu.VMEM((D, D), BF16),
            pltpu.VMEM((3 * DT, D // 2, LANES), U32),
            pltpu.VMEM((DT, D // 2, LANES), U32),
            pltpu.VMEM((DT, B_PAD + S, LANES), F32),
            pltpu.VMEM((DT, B_PAD + S, LANES), F32),
            pltpu.VMEM((S, D), BF16),
            pltpu.VMEM((M + seg, D), F32),
            pltpu.VMEM((S, D), A_x.dtype),
            pltpu.SemaphoreType.DMA((3,)),
            pltpu.SemaphoreType.DMA((4, S // B_BLK)),
            pltpu.SemaphoreType.DMA(()),
        ],
        compiler_params=pltpu.CompilerParams(vmem_limit_bytes=110 * 1024 * 1024),
    )(
        A_x.reshape(S, D), A_mem0.reshape(M, D), w_t(A_Wq), w_t(A_Wk), w_t(A_Wv),
        A_Wo.reshape(E, D), B_wqkv, B_wo, gate_w.reshape(1, D),
    )
    return out.reshape(batch, S, D)
```

```python
import functools

import jax
import jax.numpy as jnp
import jax.experimental.pallas as pl
import jax.experimental.pallas.tpu as pltpu

F32 = jnp.float32
BF16 = jnp.bfloat16
U32 = jnp.uint32
LANES, SUBLANES = 128, 8
NEG = -1000000000.0

B_HEADS, B_WIN, B_DIL = 32, 8, 2
B_PAD = 16
B_BLK = 256
ORDER = (("K", 0), ("Q", 0), ("P", 2), ("V", 0), ("S", 0), ("O", 4))
B_MM = 128
Q_MM = 128
R_LAG = 2
Q_PRE = 8
B_SUB = 16


def _nn(a, b):
    return jax.lax.dot_general(a, b, (((1,), (0,)), ((), ())), preferred_element_type=F32)


def _nt(a, b):
    return jax.lax.dot_general(a, b, (((1,), (1,)), ((), ())), preferred_element_type=F32)


def _pack(w):
    return pltpu.bitcast(w, U32)


def _unpack(w):
    return pltpu.bitcast(w, BF16)


def _iota(shape, dim):
    return jax.lax.broadcasted_iota(jnp.int32, shape, dim)


def _interleave(main, *sides):
    for n, fn in enumerate(main):
        fn()
        for side in sides:
            for extra in side[n * len(side) // len(main):(n + 1) * len(side) // len(main)]:
                extra()


def _schedule(n_pair, n_tile):
    stages = ORDER
    ops = []
    for j in range(n_pair + max(lag for _, lag in stages)):
        ops += [(op, j - lag) for op, lag in stages if 0 <= j - lag < n_pair]
    return ops + [("B", t) for t in range(n_tile)]


def _kernel(x_hbm, mem0_ref, wq_hbm, wk_hbm, wv_hbm, wo_hbm, bqkv_hbm, bwo_hbm, gate_ref,
            out_hbm,
            x_v, stage, w_v, wo_v, bqkv_raw, bwo_raw, bqkv_v, bwo_v, perm_v, wq_now, qb_v, kb_v, vb_v, ob_v,
            xpre_v, qpre_v, h_v, out_v, sem_in, sem_w, sem_out, *, seg, dh):
    S, D = x_v.shape
    M = mem0_ref.shape[0]
    L = M + seg
    E = stage.shape[1]
    DT = D // LANES
    PT = 2 * dh // LANES
    n_pair = E // (2 * dh)
    n_seg = S // seg
    n_blk = S // B_BLK
    q_tiles = E // LANES // n_blk
    r_tiles = E // LANES // (n_blk - R_LAG)
    w_hbm = (wq_hbm, wk_hbm, wv_hbm, wo_hbm)

    cp_bqkv = pltpu.make_async_copy(bqkv_hbm, bqkv_raw, sem_in.at[0])
    cp_x = pltpu.make_async_copy(x_hbm, x_v, sem_in.at[1])
    cp_bwo = pltpu.make_async_copy(bwo_hbm, bwo_raw, sem_in.at[2])

    def cp_w(m, c):
        n = (r_tiles if m else q_tiles) * LANES
        rows = pl.ds(c * n, n)
        return pltpu.make_async_copy(w_hbm[m].at[rows], stage.at[m, rows], sem_w.at[m, c])

    cp_bqkv.start()
    cp_bqkv.wait()
    cp_x.start()
    cp_w(0, 0).start()

    db = D // B_HEADS

    def interleaved(t, first, ds):
        return jnp.concatenate(
            [perm_v[t, pl.ds(first + d, B_HEADS, stride=db), :] for d in ds], axis=0).astype(BF16)

    for c in range(3 * DT):
        wt = bqkv_raw[:, c * LANES:(c + 1) * LANES].T.astype(F32)
        for t in range(DT):
            perm_v[t, c * LANES:(c + 1) * LANES, :] = wt[:, t * LANES:(t + 1) * LANES]
    per_tile = LANES // B_HEADS
    for c in range(3 * DT):
        ds = range(c % DT * per_tile, (c % DT + 1) * per_tile)
        for t in range(DT):
            bqkv_v[c, t] = _pack(interleaved(t, c // DT * D, ds))

    def b_project(xb, c):
        return _nt(xb, jnp.concatenate([_unpack(bqkv_v[c, t]) for t in range(DT)], axis=1))

    cp_x.wait()
    cp_bwo.start()
    for c in range(1, R_LAG):
        cp_w(0, c).start()

    for t in range(DT):
        kb_v[t, 0:B_PAD, :] = jnp.zeros((B_PAD, LANES), F32)
        v0 = b_project(x_v[0:B_PAD, :], 2 * DT + t)
        vb_v[t, 0:B_PAD, :] = jnp.broadcast_to(v0[0:1, :], (B_PAD, LANES))

    for s in range(0, n_seg, 2):
        tails = [x_v[e - 2 * Q_PRE:e, :].astype(F32)[Q_PRE:] for e in ((s + 1) * seg, (s + 2) * seg)]
        xpre_v[s * Q_PRE:(s + 2) * Q_PRE, :] = jnp.concatenate(tails, axis=0).astype(BF16)

    b_scale = db ** -0.5

    def window_attention(base, r):
        q = [qb_v[t, r:r + B_SUB, :] for t in range(DT)]
        pos = base + r + _iota((B_SUB, LANES), 0)

        rows = [slice(r + B_PAD - w * B_DIL, r + B_PAD - w * B_DIL + B_SUB) for w in range(B_WIN)]
        logits = []
        for w in range(B_WIN):
            acc = functools.reduce(jnp.add, [q[t] * kb_v[t, rows[w], :] for t in range(DT)])
            shift = LANES // 2
            while shift >= B_HEADS:
                acc = acc + pltpu.roll(acc, shift, 1)
                shift //= 2
            acc = acc * b_scale
            logits.append(jnp.where(pos >= w * B_DIL, acc, NEG) if w else acc)
        mx = functools.reduce(jnp.maximum, logits)
        ex = [jnp.exp(l - mx) for l in logits]
        inv = 1.0 / functools.reduce(jnp.add, ex)
        for t in range(DT):
            acc = functools.reduce(jnp.add, [ex[w] * vb_v[t, rows[w], :] for w in range(B_WIN)])
            ob_v[pl.ds(pl.multiple_of(base + r, B_SUB), B_SUB), t * LANES:(t + 1) * LANES] = acc * inv

    def retile(m, tile, t):
        rows = pl.ds(pl.multiple_of(tile * LANES, LANES), LANES)
        w = _pack(stage[m, rows, t * LANES:(t + 1) * LANES].T)
        w_v[m, tile, t * LANES // 2:(t + 1) * LANES // 2, :] = w
        return w

    def phase0(i, rest):
        @pl.when(i + R_LAG < n_blk)
        def _():
            cp_w(0, i + R_LAG).start()
            for m in range(1, 4):
                cp_w(m, i).start()

        cp_w(0, i).wait()
        if rest:
            for m in range(1, 4):
                cp_w(m, i - R_LAG).wait()

        def b_qkv(r, c):
            base = pl.multiple_of(i * B_BLK + r, B_MM)
            y = b_project(x_v[pl.ds(base, B_MM), :], c)
            if c < DT:
                qb_v[c, r:r + B_MM, :] = y
            else:
                (kb_v, vb_v)[c // DT - 1][c % DT, B_PAD + r:B_PAD + r + B_MM, :] = y

        def retile_wq(k, t):
            wq_now[k, t * LANES // 2:(t + 1) * LANES // 2, :] = retile(0, i * q_tiles + k, t)

        def a_query(r, k):
            qpre_v[i * q_tiles + k, r:r + Q_MM, :] = _nn(xpre_v[r:r + Q_MM, :], _unpack(wq_now[k]))

        def retile_wo(tile):
            rows = pl.ds(pl.multiple_of(tile * LANES, LANES), LANES)
            half = pl.ds(pl.multiple_of(tile * (LANES // 2), LANES // 2), LANES // 2)
            for t in range(DT):
                wo_v[t, half, :] = _pack(stage[3, rows, t * LANES:(t + 1) * LANES])

        task = functools.partial
        side = [task(retile_wq, k, t) for k in range(q_tiles) for t in range(DT)]
        for r in range(0, B_BLK, B_MM):
            _interleave([task(b_qkv, r, c) for c in range(3 * DT)], side)
            side = [task(window_attention, i * B_BLK, r + u) for u in range(0, B_MM, B_SUB)]
        more = []
        for k in range(r_tiles if rest else 0):
            tile = (i - R_LAG) * r_tiles + k
            more += [task(retile, m, tile, t) for m in (1, 2) for t in range(DT)] + [task(retile_wo, tile)]
        _interleave([task(a_query, r, k)
                     for r in range(0, n_seg * Q_PRE, Q_MM) for k in range(q_tiles)], side, more)
        for ref in (kb_v, vb_v):
            ref[:, 0:B_PAD, :] = ref[:, B_BLK:B_BLK + B_PAD, :]

    jax.lax.fori_loop(0, R_LAG, lambda i, c: phase0(i, False), None)
    jax.lax.fori_loop(R_LAG, n_blk, lambda i, c: phase0(i, True), None)

    cp_bwo.wait()
    for t in range(DT):
        perm_v[t, 0:D, :] = bwo_raw[:, t * LANES:(t + 1) * LANES].astype(F32)
    for t in range(DT):
        bwo_v[t] = _pack(interleaved(t, 0, range(db)))

    h_v[0:M, :] = mem0_ref[...].astype(F32)
    gate = gate_ref[...].astype(F32)
    a_scale = dh ** -0.5
    split = dh - LANES

    def step(s, carry):
        base = pl.multiple_of(s * seg, seg)
        xs = x_v[pl.ds(base, seg), :].astype(F32)
        h_v[M:L, :] = xs
        pre = pl.ds(pl.multiple_of(s * Q_PRE, Q_PRE), Q_PRE)

        lo = _iota((L, LANES), 1) < split
        zero = jnp.zeros((L, LANES), F32)
        row, col = _iota((L, 2 * L), 0), _iota((L, 2 * L), 1)
        even = col < L
        visible = (row < M) | (row >= jnp.where(even, col, col - L))

        def project(m, j):
            return [_nn(h_v[...], _unpack(w_v[m, j * PT + t])) for t in range(PT)]

        def two_heads(y):
            top = jnp.concatenate([y[0], jnp.where(lo, y[1], 0.0), zero], axis=1)
            bot = jnp.concatenate([zero, jnp.where(lo, 0.0, y[1]), y[2]], axis=1)
            return jnp.concatenate([top, bot], axis=0).astype(BF16)

        def softmax(sc):
            sc = jnp.where(visible, sc * a_scale, NEG)
            m0 = jnp.max(jnp.where(even, sc, -jnp.inf), axis=1, keepdims=True)
            m1 = jnp.max(jnp.where(even, -jnp.inf, sc), axis=1, keepdims=True)
            e = jnp.exp(sc - jnp.where(even, m0, m1))
            s0 = jnp.sum(jnp.where(even, e, 0.0), axis=1, keepdims=True)
            s1 = jnp.sum(jnp.where(even, 0.0, e), axis=1, keepdims=True)
            return e / jnp.where(even, s0, s1)

        ob = ob_v[pl.ds(base, seg), :]
        q, k, v, p, o, b, acc = {}, {}, {}, {}, {}, {}, [None] * DT
        for op, j in _schedule(n_pair, DT):
            if op == "K":
                k[j] = two_heads(project(1, j))
            elif op == "Q":
                q[j] = jnp.concatenate([
                    jnp.concatenate([_nn(h_v[0:L - Q_PRE, :], _unpack(w_v[0, c])), qpre_v[c, pre, :]], axis=0)
                    for c in range(j * PT, (j + 1) * PT)], axis=1)
            elif op == "V":
                v[j] = two_heads(project(2, j))
            elif op == "S":
                p[j] = softmax(_nt(q.pop(j), k.pop(j)))
            elif op == "P":
                o[j] = _nn(p.pop(j), v.pop(j))
            elif op == "O":
                oj = o.pop(j)
                for t in range(DT):
                    y = _nn(oj, _unpack(wo_v[t, j * dh:(j + 1) * dh, :]))
                    acc[t] = y if acc[t] is None else acc[t] + y
            else:
                b[j] = _nn(ob, _unpack(bwo_v[j]))

        g = jax.nn.sigmoid(jnp.sum(xs * gate, axis=1, keepdims=True))
        for t in range(DT):
            lanes = slice(t * LANES, (t + 1) * LANES)
            h_v[0:M, lanes] = acc[t][0:M]
            out_v[pl.ds(base, seg), lanes] = (g * acc[t][M:L] + (1.0 - g) * b[t]).astype(out_v.dtype)
        pltpu.make_async_copy(out_v.at[pl.ds(base, seg)], out_hbm.at[pl.ds(base, seg)], sem_out).start()
        return carry

    jax.lax.fori_loop(0, n_seg, step, 0)
    pltpu.make_async_copy(out_v, out_hbm, sem_out).wait()


@functools.partial(jax.jit, static_argnames=("A_seg_len",))
def pallas_gated_mix__memory_aug_recurrent_mem_tr__sliding_local_dilated__prompt_kernel(
    A_x: jax.Array,
    A_mem0: jax.Array,
    A_Wq: jax.Array,
    A_Wk: jax.Array,
    A_Wv: jax.Array,
    A_Wo: jax.Array,
    A_seg_len: int,
    B_x: jax.Array,
    B_wqkv: jax.Array,
    B_wo: jax.Array,
    gate_w: jax.Array,
):
    del B_x
    batch, S, D = A_x.shape
    _, H, dh = A_Wq.shape
    M = A_mem0.shape[1]
    E = H * dh
    seg = int(A_seg_len)
    assert batch == 1 and D % LANES == 0 and 2 * dh == 3 * LANES and H % 2 == 0
    assert S % B_BLK == 0 and S % seg == 0 and E % (S // B_BLK * LANES) == 0

    def w_t(w):
        return jnp.transpose(w, (1, 2, 0)).reshape(E, D)

    hbm = pl.BlockSpec(memory_space=pl.ANY)
    vmem = pl.BlockSpec(memory_space=pltpu.VMEM)
    DT = D // LANES
    out = pl.pallas_call(
        functools.partial(_kernel, seg=seg, dh=dh),
        out_shape=jax.ShapeDtypeStruct((S, D), A_x.dtype),
        in_specs=[hbm, vmem, hbm, hbm, hbm, hbm, hbm, hbm, vmem],
        out_specs=hbm,
        scratch_shapes=[
            pltpu.VMEM((S, D), BF16),
            pltpu.VMEM((4, E, D), BF16),
            pltpu.VMEM((3, E // LANES, D // 2, LANES), U32),
            pltpu.VMEM((DT, E // 2, LANES), U32),
            pltpu.VMEM((D, 3 * D), BF16),
            pltpu.VMEM((D, D), BF16),
            pltpu.VMEM((3 * DT, DT, LANES // 2, LANES), U32),
            pltpu.VMEM((DT, D // 2, LANES), U32),
            pltpu.VMEM((DT, 3 * D, LANES), F32),
            pltpu.VMEM((E // LANES // (S // B_BLK), D // 2, LANES), U32),
            pltpu.VMEM((DT, B_BLK, LANES), F32),
            pltpu.VMEM((DT, B_PAD + B_BLK, LANES), F32),
            pltpu.VMEM((DT, B_PAD + B_BLK, LANES), F32),
            pltpu.VMEM((S, D), F32),
            pltpu.VMEM((S // seg * Q_PRE, D), BF16),
            pltpu.VMEM((E // LANES, S // seg * Q_PRE, LANES), F32),
            pltpu.VMEM((M + seg, D), F32),
            pltpu.VMEM((S, D), A_x.dtype),
            pltpu.SemaphoreType.DMA((3,)),
            pltpu.SemaphoreType.DMA((4, S // B_BLK)),
            pltpu.SemaphoreType.DMA(()),
        ],
        compiler_params=pltpu.CompilerParams(vmem_limit_bytes=120 * 1024 * 1024),
    )(
        A_x.reshape(S, D), A_mem0.reshape(M, D), w_t(A_Wq), w_t(A_Wk), w_t(A_Wv),
        A_Wo.reshape(E, D), B_wqkv, B_wo, gate_w.reshape(1, D),
    )
    return out.reshape(batch, S, D)
```

```python
import functools

import jax
import jax.numpy as jnp
import jax.experimental.pallas as pl
import jax.experimental.pallas.tpu as pltpu

F32 = jnp.float32
BF16 = jnp.bfloat16
U32 = jnp.uint32
LANES, SUBLANES = 128, 8
NEG = -1000000000.0

B_HEADS, B_WIN, B_DIL = 32, 8, 2
B_PAD = 16
B_BLK = 256
ORDER = (("K", 0), ("Q", 0), ("P", 2), ("V", 0), ("S", 0), ("O", 4))
B_MM = 128
Q_MM = 128
UNROLL = 4
R_LAG = 2
Q_PRE = 8
B_SUB = 16


def _nn(a, b):
    return jax.lax.dot_general(a, b, (((1,), (0,)), ((), ())), preferred_element_type=F32)


def _nt(a, b):
    return jax.lax.dot_general(a, b, (((1,), (1,)), ((), ())), preferred_element_type=F32)


def _pack(w):
    return pltpu.bitcast(w, U32)


def _unpack(w):
    return pltpu.bitcast(w, BF16)


def _iota(shape, dim):
    return jax.lax.broadcasted_iota(jnp.int32, shape, dim)


def _interleave(main, *sides):
    for n, fn in enumerate(main):
        fn()
        for side in sides:
            for extra in side[n * len(side) // len(main):(n + 1) * len(side) // len(main)]:
                extra()


def _schedule(n_pair, n_tile):
    stages = ORDER
    ops = []
    for j in range(n_pair + max(lag for _, lag in stages)):
        ops += [(op, j - lag) for op, lag in stages if 0 <= j - lag < n_pair]
    return ops + [("B", t) for t in range(n_tile)]


def _kernel(x_hbm, mem0_ref, wq_hbm, wk_hbm, wv_hbm, wo_hbm, bqkv_hbm, bwo_hbm, gate_ref,
            out_hbm,
            x_v, stage, w_v, wo_v, bqkv_raw, bwo_raw, bqkv_v, bwo_v, perm_v, wq_now, qb_v, kb_v, vb_v, ob_v,
            xpre_v, qpre_v, h_v, out_v, sem_in, sem_w, sem_out, *, seg, dh):
    S, D = x_v.shape
    M = mem0_ref.shape[0]
    L = M + seg
    E = stage.shape[1]
    DT = D // LANES
    PT = 2 * dh // LANES
    n_pair = E // (2 * dh)
    n_seg = S // seg
    n_blk = S // B_BLK
    q_tiles = E // LANES // n_blk
    r_tiles = E // LANES // (n_blk - R_LAG)
    w_hbm = (wq_hbm, wk_hbm, wv_hbm, wo_hbm)

    cp_bqkv = pltpu.make_async_copy(bqkv_hbm, bqkv_raw, sem_in.at[0])
    cp_x = pltpu.make_async_copy(x_hbm, x_v, sem_in.at[1])
    cp_bwo = pltpu.make_async_copy(bwo_hbm, bwo_raw, sem_in.at[2])

    def cp_w(m, c):
        n = (r_tiles if m else q_tiles) * LANES
        rows = pl.ds(c * n, n)
        return pltpu.make_async_copy(w_hbm[m].at[rows], stage.at[m, rows], sem_w.at[m, c])

    cp_bqkv.start()
    cp_bqkv.wait()
    cp_x.start()
    cp_w(0, 0).start()

    db = D // B_HEADS

    def interleaved(t, first, ds):
        return jnp.concatenate(
            [perm_v[t, pl.ds(first + d, B_HEADS, stride=db), :] for d in ds], axis=0).astype(BF16)

    for c in range(3 * DT):
        wt = bqkv_raw[:, c * LANES:(c + 1) * LANES].T.astype(F32)
        for t in range(DT):
            perm_v[t, c * LANES:(c + 1) * LANES, :] = wt[:, t * LANES:(t + 1) * LANES]
    per_tile = LANES // B_HEADS
    for c in range(3 * DT):
        ds = range(c % DT * per_tile, (c % DT + 1) * per_tile)
        for t in range(DT):
            bqkv_v[c, t] = _pack(interleaved(t, c // DT * D, ds))

    def b_project(xb, c):
        return _nt(xb, jnp.concatenate([_unpack(bqkv_v[c, t]) for t in range(DT)], axis=1))

    cp_x.wait()
    cp_bwo.start()
    for c in range(1, R_LAG):
        cp_w(0, c).start()

    for t in range(DT):
        kb_v[t, 0:B_PAD, :] = jnp.zeros((B_PAD, LANES), F32)
        v0 = b_project(x_v[0:B_PAD, :], 2 * DT + t)
        vb_v[t, 0:B_PAD, :] = jnp.broadcast_to(v0[0:1, :], (B_PAD, LANES))

    for s in range(0, n_seg, 2):
        tails = [x_v[e - 2 * Q_PRE:e, :].astype(F32)[Q_PRE:] for e in ((s + 1) * seg, (s + 2) * seg)]
        xpre_v[s * Q_PRE:(s + 2) * Q_PRE, :] = jnp.concatenate(tails, axis=0).astype(BF16)

    b_scale = db ** -0.5

    def window_attention(base, r):
        q = [qb_v[t, r:r + B_SUB, :] for t in range(DT)]
        pos = base + r + _iota((B_SUB, LANES), 0)

        rows = [slice(r + B_PAD - w * B_DIL, r + B_PAD - w * B_DIL + B_SUB) for w in range(B_WIN)]
        logits = []
        for w in range(B_WIN):
            acc = functools.reduce(jnp.add, [q[t] * kb_v[t, rows[w], :] for t in range(DT)])
            shift = LANES // 2
            while shift >= B_HEADS:
                acc = acc + pltpu.roll(acc, shift, 1)
                shift //= 2
            acc = acc * b_scale
            logits.append(jnp.where(pos >= w * B_DIL, acc, NEG) if w else acc)
        mx = functools.reduce(jnp.maximum, logits)
        ex = [jnp.exp(l - mx) for l in logits]
        inv = 1.0 / functools.reduce(jnp.add, ex)
        for t in range(DT):
            acc = functools.reduce(jnp.add, [ex[w] * vb_v[t, rows[w], :] for w in range(B_WIN)])
            ob_v[pl.ds(pl.multiple_of(base + r, B_SUB), B_SUB), t * LANES:(t + 1) * LANES] = acc * inv

    def retile(m, tile, t):
        rows = pl.ds(pl.multiple_of(tile * LANES, LANES), LANES)
        w = _pack(stage[m, rows, t * LANES:(t + 1) * LANES].T)
        w_v[m, tile, t * LANES // 2:(t + 1) * LANES // 2, :] = w
        return w

    def phase0(i, rest):
        @pl.when(i + R_LAG < n_blk)
        def _():
            cp_w(0, i + R_LAG).start()
            for m in range(1, 4):
                cp_w(m, i).start()

        cp_w(0, i).wait()
        if rest:
            for m in range(1, 4):
                cp_w(m, i - R_LAG).wait()

        def b_qkv(r, c):
            base = pl.multiple_of(i * B_BLK + r, B_MM)
            y = b_project(x_v[pl.ds(base, B_MM), :], c)
            if c < DT:
                qb_v[c, r:r + B_MM, :] = y
            else:
                (kb_v, vb_v)[c // DT - 1][c % DT, B_PAD + r:B_PAD + r + B_MM, :] = y

        def retile_wq(k, t):
            wq_now[k, t * LANES // 2:(t + 1) * LANES // 2, :] = retile(0, i * q_tiles + k, t)

        def a_query(r, k):
            qpre_v[i * q_tiles + k, r:r + Q_MM, :] = _nn(xpre_v[r:r + Q_MM, :], _unpack(wq_now[k]))

        def retile_wo(tile):
            rows = pl.ds(pl.multiple_of(tile * LANES, LANES), LANES)
            half = pl.ds(pl.multiple_of(tile * (LANES // 2), LANES // 2), LANES // 2)
            for t in range(DT):
                wo_v[t, half, :] = _pack(stage[3, rows, t * LANES:(t + 1) * LANES])

        task = functools.partial
        side = [task(retile_wq, k, t) for k in range(q_tiles) for t in range(DT)]
        for r in range(0, B_BLK, B_MM):
            _interleave([task(b_qkv, r, c) for c in range(3 * DT)], side)
            side = [task(window_attention, i * B_BLK, r + u) for u in range(0, B_MM, B_SUB)]
        more = []
        for k in range(r_tiles if rest else 0):
            tile = (i - R_LAG) * r_tiles + k
            more += [task(retile, m, tile, t) for m in (1, 2) for t in range(DT)] + [task(retile_wo, tile)]
        _interleave([task(a_query, r, k)
                     for r in range(0, n_seg * Q_PRE, Q_MM) for k in range(q_tiles)], side, more)
        for ref in (kb_v, vb_v):
            ref[:, 0:B_PAD, :] = ref[:, B_BLK:B_BLK + B_PAD, :]

    jax.lax.fori_loop(0, R_LAG, lambda i, c: phase0(i, False), None)
    jax.lax.fori_loop(R_LAG, n_blk, lambda i, c: phase0(i, True), None)

    cp_bwo.wait()
    for t in range(DT):
        perm_v[t, 0:D, :] = bwo_raw[:, t * LANES:(t + 1) * LANES].astype(F32)
    for t in range(DT):
        bwo_v[t] = _pack(interleaved(t, 0, range(db)))

    h_v[0:M, :] = mem0_ref[...].astype(F32)
    gate = gate_ref[...].astype(F32).reshape(1, D)
    a_scale = dh ** -0.5
    split = dh - LANES

    def segment(s):
        base = pl.multiple_of(s * seg, seg)
        xs = x_v[pl.ds(base, seg), :].astype(F32)
        h_v[M:L, :] = xs
        pre = pl.ds(pl.multiple_of(s * Q_PRE, Q_PRE), Q_PRE)

        lo = _iota((L, LANES), 1) < split
        zero = jnp.zeros((L, LANES), F32)
        row, col = _iota((L, 2 * L), 0), _iota((L, 2 * L), 1)
        even = col < L
        visible = (row < M) | (row >= jnp.where(even, col, col - L))

        def project(m, j):
            return [_nn(h_v[...], _unpack(w_v[m, j * PT + t])) for t in range(PT)]

        def two_heads(y):
            top = jnp.concatenate([y[0], jnp.where(lo, y[1], 0.0), zero], axis=1)
            bot = jnp.concatenate([zero, jnp.where(lo, 0.0, y[1]), y[2]], axis=1)
            return jnp.concatenate([top, bot], axis=0).astype(BF16)

        def softmax(sc):
            sc = jnp.where(visible, sc * a_scale, NEG)
            m0 = jnp.max(jnp.where(even, sc, -jnp.inf), axis=1, keepdims=True)
            m1 = jnp.max(jnp.where(even, -jnp.inf, sc), axis=1, keepdims=True)
            e = jnp.exp(sc - jnp.where(even, m0, m1))
            s0 = jnp.sum(jnp.where(even, e, 0.0), axis=1, keepdims=True)
            s1 = jnp.sum(jnp.where(even, 0.0, e), axis=1, keepdims=True)
            return e / jnp.where(even, s0, s1)

        ob = ob_v[pl.ds(base, seg), :]
        q, k, v, p, o, b, acc = {}, {}, {}, {}, {}, {}, [None] * DT
        for op, j in _schedule(n_pair, DT):
            if op == "K":
                k[j] = two_heads(project(1, j))
            elif op == "Q":
                q[j] = jnp.concatenate([
                    jnp.concatenate([_nn(h_v[0:L - Q_PRE, :], _unpack(w_v[0, c])), qpre_v[c, pre, :]], axis=0)
                    for c in range(j * PT, (j + 1) * PT)], axis=1)
            elif op == "V":
                v[j] = two_heads(project(2, j))
            elif op == "S":
                p[j] = softmax(_nt(q.pop(j), k.pop(j)))
            elif op == "P":
                o[j] = _nn(p.pop(j), v.pop(j))
            elif op == "O":
                oj = o.pop(j)
                for t in range(DT):
                    y = _nn(oj, _unpack(wo_v[t, j * dh:(j + 1) * dh, :]))
                    acc[t] = y if acc[t] is None else acc[t] + y
            else:
                b[j] = _nn(ob, _unpack(bwo_v[j]))

        g = jax.nn.sigmoid(jnp.sum(xs * gate, axis=1, keepdims=True))
        for t in range(DT):
            lanes = slice(t * LANES, (t + 1) * LANES)
            h_v[0:M, lanes] = acc[t][0:M]
            out_v[pl.ds(base, seg), lanes] = (g * acc[t][M:L] + (1.0 - g) * b[t]).astype(out_v.dtype)

    def step(i, carry):
        for u in range(UNROLL):
            segment(i * UNROLL + u)
        rows = pl.ds(pl.multiple_of(i * (UNROLL * seg), UNROLL * seg), UNROLL * seg)
        pltpu.make_async_copy(out_v.at[rows], out_hbm.at[rows], sem_out).start()
        return carry

    jax.lax.fori_loop(0, n_seg // UNROLL, step, 0)
    pltpu.make_async_copy(out_v, out_hbm, sem_out).wait()


@functools.partial(jax.jit, static_argnames=("A_seg_len",))
def pallas_gated_mix__memory_aug_recurrent_mem_tr__sliding_local_dilated__prompt_kernel(
    A_x: jax.Array,
    A_mem0: jax.Array,
    A_Wq: jax.Array,
    A_Wk: jax.Array,
    A_Wv: jax.Array,
    A_Wo: jax.Array,
    A_seg_len: int,
    B_x: jax.Array,
    B_wqkv: jax.Array,
    B_wo: jax.Array,
    gate_w: jax.Array,
):
    del B_x
    batch, S, D = A_x.shape
    _, H, dh = A_Wq.shape
    M = A_mem0.shape[1]
    E = H * dh
    seg = int(A_seg_len)
    assert batch == 1 and D % LANES == 0 and 2 * dh == 3 * LANES and H % 2 == 0
    assert S % B_BLK == 0 and S % seg == 0 and E % (S // B_BLK * LANES) == 0

    def w_t(w):
        return jnp.transpose(w, (1, 2, 0)).reshape(E, D)

    hbm = pl.BlockSpec(memory_space=pl.ANY)
    vmem = pl.BlockSpec(memory_space=pltpu.VMEM)
    DT = D // LANES
    out = pl.pallas_call(
        functools.partial(_kernel, seg=seg, dh=dh),
        out_shape=jax.ShapeDtypeStruct((S, D), A_x.dtype),
        in_specs=[hbm, vmem, hbm, hbm, hbm, hbm, hbm, hbm, vmem],
        out_specs=hbm,
        scratch_shapes=[
            pltpu.VMEM((S, D), BF16),
            pltpu.VMEM((4, E, D), BF16),
            pltpu.VMEM((3, E // LANES, D // 2, LANES), U32),
            pltpu.VMEM((DT, E // 2, LANES), U32),
            pltpu.VMEM((D, 3 * D), BF16),
            pltpu.VMEM((D, D), BF16),
            pltpu.VMEM((3 * DT, DT, LANES // 2, LANES), U32),
            pltpu.VMEM((DT, D // 2, LANES), U32),
            pltpu.VMEM((DT, 3 * D, LANES), F32),
            pltpu.VMEM((E // LANES // (S // B_BLK), D // 2, LANES), U32),
            pltpu.VMEM((DT, B_BLK, LANES), F32),
            pltpu.VMEM((DT, B_PAD + B_BLK, LANES), F32),
            pltpu.VMEM((DT, B_PAD + B_BLK, LANES), F32),
            pltpu.VMEM((S, D), F32),
            pltpu.VMEM((S // seg * Q_PRE, D), BF16),
            pltpu.VMEM((E // LANES, S // seg * Q_PRE, LANES), F32),
            pltpu.VMEM((M + seg, D), F32),
            pltpu.VMEM((S, D), A_x.dtype),
            pltpu.SemaphoreType.DMA((3,)),
            pltpu.SemaphoreType.DMA((4, S // B_BLK)),
            pltpu.SemaphoreType.DMA(()),
        ],
        compiler_params=pltpu.CompilerParams(vmem_limit_bytes=120 * 1024 * 1024),
    )(
        A_x.reshape(S, D), A_mem0.reshape(M, D), w_t(A_Wq), w_t(A_Wk), w_t(A_Wv),
        A_Wo.reshape(E, D), B_wqkv, B_wo, gate_w,
    )
    return out.reshape(batch, S, D)
```

```python
import functools

import jax
import jax.numpy as jnp
import jax.experimental.pallas as pl
import jax.experimental.pallas.tpu as pltpu

F32 = jnp.float32
BF16 = jnp.bfloat16
U32 = jnp.uint32
LANES, SUBLANES = 128, 8
NEG = -1000000000.0

B_HEADS, B_WIN, B_DIL = 32, 8, 2
B_PAD = 16
B_BLK = 256
ORDER = (("K", 0), ("Q", 0), ("P", 2), ("V", 0), ("S", 0), ("O", 4))
B_MM = 128
SPLIT = 50
UNROLL = 2
Q_PRE = 8
B_SUB = 32


def _nn(a, b):
    return jax.lax.dot_general(a, b, (((1,), (0,)), ((), ())), preferred_element_type=F32)


def _nt(a, b):
    return jax.lax.dot_general(a, b, (((1,), (1,)), ((), ())), preferred_element_type=F32)


def _pack(w):
    return pltpu.bitcast(w, U32)


def _unpack(w):
    return pltpu.bitcast(w, BF16)


def _iota(shape, dim):
    return jax.lax.broadcasted_iota(jnp.int32, shape, dim)


def _interleave(main, *sides):
    for n, fn in enumerate(main):
        fn()
        for side in sides:
            for extra in side[n * len(side) // len(main):(n + 1) * len(side) // len(main)]:
                extra()


def _schedule(n_pair, n_tile):
    stages = ORDER
    ops = []
    for j in range(n_pair + max(lag for _, lag in stages)):
        ops += [(op, j - lag) for op, lag in stages if 0 <= j - lag < n_pair]
    return ops + [("B", t) for t in range(n_tile)]


def _kernel(x_hbm, mem0_ref, wq_hbm, wk_hbm, wv_hbm, wo_hbm, bqkv_hbm, bwo_hbm, gate_ref,
            out_hbm,
            x_v, stage, w_v, wo_v, bqkv_raw, bwo_raw, bqkv_v, bwo_v, perm_v, qb_v, kb_v, vb_v, ob_v,
            xpre_v, qpre_v, h_v, out_v, sem_in, sem_w, sem_out, *, seg, dh):
    S, D = x_v.shape
    M = mem0_ref.shape[0]
    L = M + seg
    E = stage.shape[1]
    DT = D // LANES
    PT = 2 * dh // LANES
    n_pair = E // (2 * dh)
    n_seg = S // seg
    n_blk = S // B_BLK
    q_tiles = E // LANES // n_blk
    r_tiles = E // LANES // (n_blk - 2)
    w_hbm = (wq_hbm, wk_hbm, wv_hbm, wo_hbm)

    cp_bqkv = pltpu.make_async_copy(bqkv_hbm, bqkv_raw, sem_in.at[0])
    head, tail = pl.ds(0, B_BLK), pl.ds(B_BLK, S - B_BLK)
    cp_x0 = pltpu.make_async_copy(x_hbm.at[head], x_v.at[head], sem_in.at[1])
    cp_x1 = pltpu.make_async_copy(x_hbm.at[tail], x_v.at[tail], sem_in.at[3])
    cp_bwo = pltpu.make_async_copy(bwo_hbm, bwo_raw, sem_in.at[2])

    def cp_w(m, c):
        n = (r_tiles if m else q_tiles) * LANES
        rows = pl.ds(c * n, n)
        return pltpu.make_async_copy(w_hbm[m].at[rows], stage.at[m, rows], sem_w.at[m, c])

    cp_bqkv.start()
    cp_x0.start()
    cp_bqkv.wait()
    cp_x1.start()
    cp_w(0, 0).start()

    db = D // B_HEADS

    def interleaved(t, first, ds):
        return jnp.concatenate(
            [perm_v[t, pl.ds(first + d, B_HEADS, stride=db), :] for d in ds], axis=0).astype(BF16)

    for c in range(3 * DT):
        wt = bqkv_raw[:, c * LANES:(c + 1) * LANES].T.astype(F32)
        for t in range(DT):
            perm_v[t, c * LANES:(c + 1) * LANES, :] = wt[:, t * LANES:(t + 1) * LANES]
    per_tile = LANES // B_HEADS
    for c in range(3 * DT):
        ds = range(c % DT * per_tile, (c % DT + 1) * per_tile)
        for t in range(DT):
            bqkv_v[c, t] = _pack(interleaved(t, c // DT * D, ds))

    def b_project(xb, c):
        return _nt(xb, jnp.concatenate([_unpack(bqkv_v[c, t]) for t in range(DT)], axis=1))

    b_scale = db ** -0.5

    def window_attention(base, r):
        q = [qb_v[t, r:r + B_SUB, :] for t in range(DT)]
        pos = base + r + _iota((B_SUB, LANES), 0)

        rows = [slice(r + B_PAD - w * B_DIL, r + B_PAD - w * B_DIL + B_SUB) for w in range(B_WIN)]
        logits = []
        for w in range(B_WIN):
            acc = functools.reduce(jnp.add, [q[t] * kb_v[t, rows[w], :] for t in range(DT)])
            shift = LANES // 2
            while shift >= B_HEADS:
                acc = acc + pltpu.roll(acc, shift, 1)
                shift //= 2
            acc = acc * b_scale
            logits.append(jnp.where(pos >= w * B_DIL, acc, NEG) if w else acc)
        mx = functools.reduce(jnp.maximum, logits)
        ex = [jnp.exp(l - mx) for l in logits]
        inv = 1.0 / functools.reduce(jnp.add, ex)
        for t in range(DT):
            acc = functools.reduce(jnp.add, [ex[w] * vb_v[t, rows[w], :] for w in range(B_WIN)])
            ob_v[pl.ds(pl.multiple_of(base + r, B_SUB), B_SUB), t * LANES:(t + 1) * LANES] = acc * inv

    task = functools.partial

    def b_qkv(blk, r, c):
        y = b_project(x_v[pl.ds(pl.multiple_of(blk * B_BLK + r, B_MM), B_MM), :], c)
        if c < DT:
            qb_v[c, r:r + B_MM, :] = y
        else:
            (kb_v, vb_v)[c // DT - 1][c % DT, B_PAD + r:B_PAD + r + B_MM, :] = y

    def b_attend(blk, r):
        return [task(window_attention, blk * B_BLK, r + u) for u in range(0, B_MM, B_SUB)]

    def b_block(blk, side, first=False):
        for r in range(0, B_BLK, B_MM):
            _interleave([task(b_qkv, blk, r, c) for c in range(3 * DT)], side)
            if first and r == 0:
                kb_v[:, 0:B_PAD, :] = jnp.zeros((DT, B_PAD, LANES), F32)
                for t in range(DT):
                    vb_v[t, 0:B_PAD, :] = jnp.broadcast_to(vb_v[t, B_PAD:B_PAD + 1, :], (B_PAD, LANES))
            side = b_attend(blk, r)

    def slab(tile):
        return pl.ds(pl.multiple_of(tile * LANES, LANES), LANES)

    def a_queries(i, side):
        def one(r, tile):
            qpre_v[tile, r:r + B_MM, :] = _nt(xpre_v[r:r + B_MM, :], stage[0, slab(tile), :])

        _interleave([task(one, r, i * q_tiles + k) for k in range(q_tiles)
                     for r in range(0, n_seg * Q_PRE, B_MM)], b_attend(i, B_BLK - B_MM), side)
        for ref in (kb_v, vb_v):
            ref[:, 0:B_PAD, :] = ref[:, B_BLK:B_BLK + B_PAD, :]

    def retile(m, tile, t):
        w = stage[m, slab(tile), t * LANES:(t + 1) * LANES]
        if m < 3:
            w_v[m, tile, t * LANES // 2:(t + 1) * LANES // 2, :] = _pack(w.T)
        else:
            wo_v[t, pl.ds(pl.multiple_of(tile * (LANES // 2), LANES // 2), LANES // 2), :] = _pack(w)

    def retile_q(i):
        return [task(retile, 0, i * q_tiles + k, t) for k in range(q_tiles) for t in range(DT)]

    def phase0(i, carry):
        cp_w(0, i + 1).start()

        @pl.when(i + 2 < n_blk)
        def _():
            cp_w(2, i).start()
            cp_w(3, i).start()

        @pl.when(i + 3 < n_blk)
        def _():
            cp_w(1, i + 1).start()

        cp_w(0, i).wait()
        for m in range(1, 4):
            cp_w(m, i - 1).wait()
        side = retile_q(i) + [task(retile, m, (i - 1) * r_tiles + k, t)
                              for k in range(r_tiles) for t in range(DT) for m in range(1, 4)]
        n = len(side) * SPLIT // 100
        a_queries(i, side[:n])
        b_block(i + 1, side[n:])

    cp_x0.wait()
    cp_w(0, 1).start()
    b_block(0, [], first=True)
    for m in range(1, 4):
        cp_w(m, 0).start()
    cp_x1.wait()

    for s in range(0, n_seg, 2):
        tails = [x_v[e - 2 * Q_PRE:e, :].astype(F32)[Q_PRE:] for e in ((s + 1) * seg, (s + 2) * seg)]
        xpre_v[s * Q_PRE:(s + 2) * Q_PRE, :] = jnp.concatenate(tails, axis=0).astype(BF16)

    cp_w(0, 0).wait()
    a_queries(0, [])
    cp_w(1, 1).start()
    b_block(1, retile_q(0))
    jax.lax.fori_loop(1, n_blk - 1, phase0, None)
    cp_bwo.start()
    cp_w(0, n_blk - 1).wait()
    a_queries(n_blk - 1, retile_q(n_blk - 1))

    cp_bwo.wait()
    for t in range(DT):
        perm_v[t, 0:D, :] = bwo_raw[:, t * LANES:(t + 1) * LANES].astype(F32)
    for t in range(DT):
        bwo_v[t] = _pack(interleaved(t, 0, range(db)))

    h_v[0:M, :] = mem0_ref[...].astype(F32)
    gate = gate_ref[...].astype(F32).reshape(1, D)
    a_scale = dh ** -0.5
    split = dh - LANES

    def segment(s):
        base = pl.multiple_of(s * seg, seg)
        xs = x_v[pl.ds(base, seg), :].astype(F32)
        h_v[M:L, :] = xs
        pre = pl.ds(pl.multiple_of(s * Q_PRE, Q_PRE), Q_PRE)

        lo = _iota((L, LANES), 1) < split
        zero = jnp.zeros((L, LANES), F32)
        row, col = _iota((L, 2 * L), 0), _iota((L, 2 * L), 1)
        even = col < L
        visible = (row < M) | (row >= jnp.where(even, col, col - L))

        def project(m, j):
            return [_nn(h_v[...], _unpack(w_v[m, j * PT + t])) for t in range(PT)]

        def two_heads(y):
            top = jnp.concatenate([y[0], jnp.where(lo, y[1], 0.0), zero], axis=1)
            bot = jnp.concatenate([zero, jnp.where(lo, 0.0, y[1]), y[2]], axis=1)
            return jnp.concatenate([top, bot], axis=0).astype(BF16)

        def softmax(sc):
            sc = jnp.where(visible, sc * a_scale, NEG)
            m0 = jnp.max(jnp.where(even, sc, -jnp.inf), axis=1, keepdims=True)
            m1 = jnp.max(jnp.where(even, -jnp.inf, sc), axis=1, keepdims=True)
            e = jnp.exp(sc - jnp.where(even, m0, m1))
            s0 = jnp.sum(jnp.where(even, e, 0.0), axis=1, keepdims=True)
            s1 = jnp.sum(jnp.where(even, 0.0, e), axis=1, keepdims=True)
            return e / jnp.where(even, s0, s1)

        ob = ob_v[pl.ds(base, seg), :]
        q, k, v, p, o, b, acc = {}, {}, {}, {}, {}, {}, [None] * DT
        for op, j in _schedule(n_pair, DT):
            if op == "K":
                k[j] = two_heads(project(1, j))
            elif op == "Q":
                q[j] = jnp.concatenate([
                    jnp.concatenate([_nn(h_v[0:L - Q_PRE, :], _unpack(w_v[0, c])), qpre_v[c, pre, :]], axis=0)
                    for c in range(j * PT, (j + 1) * PT)], axis=1)
            elif op == "V":
                v[j] = two_heads(project(2, j))
            elif op == "S":
                p[j] = softmax(_nt(q.pop(j), k.pop(j)))
            elif op == "P":
                o[j] = _nn(p.pop(j), v.pop(j))
            elif op == "O":
                oj = o.pop(j)
                for t in range(DT):
                    y = _nn(oj, _unpack(wo_v[t, j * dh:(j + 1) * dh, :]))
                    acc[t] = y if acc[t] is None else acc[t] + y
            else:
                b[j] = _nn(ob, _unpack(bwo_v[j]))

        g = jax.nn.sigmoid(jnp.sum(xs * gate, axis=1, keepdims=True))
        for t in range(DT):
            lanes = slice(t * LANES, (t + 1) * LANES)
            h_v[0:M, lanes] = acc[t][0:M]
            out_v[pl.ds(base, seg), lanes] = (g * acc[t][M:L] + (1.0 - g) * b[t]).astype(out_v.dtype)

    def step(i, carry):
        for u in range(UNROLL):
            segment(i * UNROLL + u)
        rows = pl.ds(pl.multiple_of(i * (UNROLL * seg), UNROLL * seg), UNROLL * seg)
        pltpu.make_async_copy(out_v.at[rows], out_hbm.at[rows], sem_out).start()
        return carry

    jax.lax.fori_loop(0, n_seg // UNROLL, step, 0)
    pltpu.make_async_copy(out_v, out_hbm, sem_out).wait()


@functools.partial(jax.jit, static_argnames=("A_seg_len",))
def pallas_gated_mix__memory_aug_recurrent_mem_tr__sliding_local_dilated__prompt_kernel(
    A_x: jax.Array,
    A_mem0: jax.Array,
    A_Wq: jax.Array,
    A_Wk: jax.Array,
    A_Wv: jax.Array,
    A_Wo: jax.Array,
    A_seg_len: int,
    B_x: jax.Array,
    B_wqkv: jax.Array,
    B_wo: jax.Array,
    gate_w: jax.Array,
):
    del B_x
    batch, S, D = A_x.shape
    _, H, dh = A_Wq.shape
    M = A_mem0.shape[1]
    E = H * dh
    seg = int(A_seg_len)
    assert batch == 1 and D % LANES == 0 and 2 * dh == 3 * LANES and H % 2 == 0
    assert S % B_BLK == 0 and S % seg == 0 and E % (S // B_BLK * LANES) == 0

    def w_t(w):
        return jnp.transpose(w, (1, 2, 0)).reshape(E, D)

    hbm = pl.BlockSpec(memory_space=pl.ANY)
    vmem = pl.BlockSpec(memory_space=pltpu.VMEM)
    DT = D // LANES
    out = pl.pallas_call(
        functools.partial(_kernel, seg=seg, dh=dh),
        out_shape=jax.ShapeDtypeStruct((S, D), A_x.dtype),
        in_specs=[hbm, vmem, hbm, hbm, hbm, hbm, hbm, hbm, vmem],
        out_specs=hbm,
        scratch_shapes=[
            pltpu.VMEM((S, D), BF16),
            pltpu.VMEM((4, E, D), BF16),
            pltpu.VMEM((3, E // LANES, D // 2, LANES), U32),
            pltpu.VMEM((DT, E // 2, LANES), U32),
            pltpu.VMEM((D, 3 * D), BF16),
            pltpu.VMEM((D, D), BF16),
            pltpu.VMEM((3 * DT, DT, LANES // 2, LANES), U32),
            pltpu.VMEM((DT, D // 2, LANES), U32),
            pltpu.VMEM((DT, 3 * D, LANES), F32),
            pltpu.VMEM((DT, B_BLK, LANES), F32),
            pltpu.VMEM((DT, B_PAD + B_BLK, LANES), F32),
            pltpu.VMEM((DT, B_PAD + B_BLK, LANES), F32),
            pltpu.VMEM((S, D), F32),
            pltpu.VMEM((S // seg * Q_PRE, D), BF16),
            pltpu.VMEM((E // LANES, S // seg * Q_PRE, LANES), F32),
            pltpu.VMEM((M + seg, D), F32),
            pltpu.VMEM((S, D), A_x.dtype),
            pltpu.SemaphoreType.DMA((4,)),
            pltpu.SemaphoreType.DMA((4, S // B_BLK)),
            pltpu.SemaphoreType.DMA(()),
        ],
        compiler_params=pltpu.CompilerParams(vmem_limit_bytes=120 * 1024 * 1024),
    )(
        A_x.reshape(S, D), A_mem0.reshape(M, D), w_t(A_Wq), w_t(A_Wk), w_t(A_Wv),
        A_Wo.reshape(E, D), B_wqkv, B_wo, gate_w,
    )
    return out.reshape(batch, S, D)
```

```python
import functools

import jax
import jax.numpy as jnp
import jax.experimental.pallas as pl
import jax.experimental.pallas.tpu as pltpu

F32 = jnp.float32
BF16 = jnp.bfloat16
U32 = jnp.uint32
LANES, SUBLANES = 128, 8
NEG = -1000000000.0

B_HEADS, B_WIN, B_DIL = 32, 8, 2
B_PAD = 16
B_BLK = 256
ORDER = (("K", 0), ("Q", 0), ("P", 2), ("V", 0), ("S", 0), ("O", 4))
B_MM = 128
SPLIT = 50
UNROLL = 2
B_EARLY = 2
Q_PRE = 8
B_SUB = 32


def _nn(a, b):
    return jax.lax.dot_general(a, b, (((1,), (0,)), ((), ())), preferred_element_type=F32)


def _nt(a, b):
    return jax.lax.dot_general(a, b, (((1,), (1,)), ((), ())), preferred_element_type=F32)


def _pack(w):
    return pltpu.bitcast(w, U32)


def _unpack(w):
    return pltpu.bitcast(w, BF16)


def _iota(shape, dim):
    return jax.lax.broadcasted_iota(jnp.int32, shape, dim)


def _interleave(main, *sides):
    for n, fn in enumerate(main):
        fn()
        for side in sides:
            for extra in side[n * len(side) // len(main):(n + 1) * len(side) // len(main)]:
                extra()


def _schedule(n_pair, n_tile):
    stages = ORDER
    ops = []
    for j in range(n_pair + max(lag for _, lag in stages)):
        ops += [(op, j - lag) for op, lag in stages if 0 <= j - lag < n_pair]
    at = ops.index(("P", n_pair - 1))
    fill = [("B", t) for t in range(n_tile)]
    return ops[:at] + fill[:B_EARLY] + ops[at:] + fill[B_EARLY:]


def _kernel(x_hbm, mem0_hbm, wq_hbm, wk_hbm, wv_hbm, wo_hbm, bqkv_hbm, bwo_hbm, gate_hbm,
            out_hbm,
            x_v, stage, w_v, wo_v, bqkv_raw, bwo_raw, bqkv_v, bwo_v, perm_v, qb_v, kb_v, vb_v, ob_v,
            xpre_v, qpre_v, h_v, out_v, mem0_v, gate_v, sem_in, sem_w, sem_out, *, seg, dh):
    S, D = x_v.shape
    M = mem0_v.shape[0]
    L = M + seg
    E = stage.shape[1]
    DT = D // LANES
    PT = 2 * dh // LANES
    n_pair = E // (2 * dh)
    n_seg = S // seg
    n_blk = S // B_BLK
    q_tiles = E // LANES // n_blk
    r_tiles = E // LANES // (n_blk - 2)
    w_hbm = (wq_hbm, wk_hbm, wv_hbm, wo_hbm)

    cp_bqkv = pltpu.make_async_copy(bqkv_hbm, bqkv_raw, sem_in.at[0])
    head, tail = pl.ds(0, B_BLK), pl.ds(B_BLK, S - B_BLK)
    cp_x0 = pltpu.make_async_copy(x_hbm.at[head], x_v.at[head], sem_in.at[1])
    cp_x1 = pltpu.make_async_copy(x_hbm.at[tail], x_v.at[tail], sem_in.at[2])
    cp_late = [pltpu.make_async_copy(src, dst, sem_in.at[3 + n])
               for n, (src, dst) in enumerate(((bwo_hbm, bwo_raw), (mem0_hbm, mem0_v), (gate_hbm, gate_v)))]

    def cp_w(m, c):
        n = (r_tiles if m else q_tiles) * LANES
        rows = pl.ds(c * n, n)
        return pltpu.make_async_copy(w_hbm[m].at[rows], stage.at[m, rows], sem_w.at[m, c])

    cp_bqkv.start()
    cp_x0.start()
    cp_x0.wait()
    cp_bqkv.wait()
    cp_x1.start()
    cp_w(0, 0).start()

    db = D // B_HEADS

    def interleaved(t, first, ds):
        return jnp.concatenate(
            [perm_v[t, pl.ds(first + d, B_HEADS, stride=db), :] for d in ds], axis=0).astype(BF16)

    def b_transpose(c):
        wt = bqkv_raw[:, c * LANES:(c + 1) * LANES].T.astype(F32)
        for t in range(DT):
            perm_v[t, c * LANES:(c + 1) * LANES, :] = wt[:, t * LANES:(t + 1) * LANES]

    def b_gather(c):
        per_tile = LANES // B_HEADS
        ds = range(c % DT * per_tile, (c % DT + 1) * per_tile)
        for t in range(DT):
            bqkv_v[c, t] = _pack(interleaved(t, c // DT * D, ds))

    def b_project(xb, c):
        return _nt(xb, jnp.concatenate([_unpack(bqkv_v[c, t]) for t in range(DT)], axis=1))

    b_scale = db ** -0.5

    def window_attention(base, r):
        q = [qb_v[t, r:r + B_SUB, :] for t in range(DT)]
        pos = base + r + _iota((B_SUB, LANES), 0)

        rows = [slice(r + B_PAD - w * B_DIL, r + B_PAD - w * B_DIL + B_SUB) for w in range(B_WIN)]
        logits = []
        for w in range(B_WIN):
            acc = functools.reduce(jnp.add, [q[t] * kb_v[t, rows[w], :] for t in range(DT)])
            shift = LANES // 2
            while shift >= B_HEADS:
                acc = acc + pltpu.roll(acc, shift, 1)
                shift //= 2
            acc = acc * b_scale
            logits.append(jnp.where(pos >= w * B_DIL, acc, NEG) if w else acc)
        mx = functools.reduce(jnp.maximum, logits)
        ex = [jnp.exp(l - mx) for l in logits]
        inv = 1.0 / functools.reduce(jnp.add, ex)
        for t in range(DT):
            acc = functools.reduce(jnp.add, [ex[w] * vb_v[t, rows[w], :] for w in range(B_WIN)])
            ob_v[pl.ds(pl.multiple_of(base + r, B_SUB), B_SUB), t * LANES:(t + 1) * LANES] = acc * inv

    task = functools.partial

    def b_qkv(blk, r, c):
        y = b_project(x_v[pl.ds(pl.multiple_of(blk * B_BLK + r, B_MM), B_MM), :], c)
        if c < DT:
            qb_v[c, r:r + B_MM, :] = y
        else:
            (kb_v, vb_v)[c // DT - 1][c % DT, B_PAD + r:B_PAD + r + B_MM, :] = y

    def b_attend(blk, r):
        return [task(window_attention, blk * B_BLK, r + u) for u in range(0, B_MM, B_SUB)]

    def b_block(blk, side, first=False):
        for r in range(0, B_BLK, B_MM):
            _interleave([task(b_qkv, blk, r, c) for c in range(3 * DT)], side)
            if first and r == 0:
                kb_v[:, 0:B_PAD, :] = jnp.zeros((DT, B_PAD, LANES), F32)
                for t in range(DT):
                    vb_v[t, 0:B_PAD, :] = jnp.broadcast_to(vb_v[t, B_PAD:B_PAD + 1, :], (B_PAD, LANES))
            side = b_attend(blk, r)

    def slab(tile):
        return pl.ds(pl.multiple_of(tile * LANES, LANES), LANES)

    def a_queries(i, side):
        def one(r, tile):
            qpre_v[tile, r:r + B_MM, :] = _nt(xpre_v[r:r + B_MM, :], stage[0, slab(tile), :])

        _interleave([task(one, r, i * q_tiles + k) for k in range(q_tiles)
                     for r in range(0, n_seg * Q_PRE, B_MM)], b_attend(i, B_BLK - B_MM), side)
        for ref in (kb_v, vb_v):
            ref[:, 0:B_PAD, :] = ref[:, B_BLK:B_BLK + B_PAD, :]

    def retile(m, tile, t):
        w = stage[m, slab(tile), t * LANES:(t + 1) * LANES]
        if m < 3:
            w_v[m, tile, t * LANES // 2:(t + 1) * LANES // 2, :] = _pack(w.T)
        else:
            wo_v[t, pl.ds(pl.multiple_of(tile * (LANES // 2), LANES // 2), LANES // 2), :] = _pack(w)

    def retile_q(i):
        return [task(retile, 0, i * q_tiles + k, t) for k in range(q_tiles) for t in range(DT)]

    def phase0(i, carry):
        cp_w(0, i + 1).start()

        @pl.when(i + 2 < n_blk)
        def _():
            cp_w(2, i).start()
            cp_w(3, i).start()

        @pl.when(i + 3 < n_blk)
        def _():
            cp_w(1, i + 1).start()

        cp_w(0, i).wait()
        for m in range(1, 4):
            cp_w(m, i - 1).wait()
        side = retile_q(i) + [task(retile, m, (i - 1) * r_tiles + k, t)
                              for k in range(r_tiles) for t in range(DT) for m in range(1, 4)]
        n = len(side) * SPLIT // 100
        a_queries(i, side[:n])
        b_block(i + 1, side[n:])

    prep = [task(fn, m * DT + t) for m in range(3) for fn in (b_transpose, b_gather) for t in range(DT)]
    for fn in prep[:2 * DT]:
        fn()
    cp_w(0, 1).start()
    b_block(0, prep[2 * DT:] + [lambda: None] * (2 * DT), first=True)
    for m in range(1, 4):
        cp_w(m, 0).start()
    cp_x1.wait()

    for s in range(0, n_seg, 2):
        tails = [x_v[e - 2 * Q_PRE:e, :].astype(F32)[Q_PRE:] for e in ((s + 1) * seg, (s + 2) * seg)]
        xpre_v[s * Q_PRE:(s + 2) * Q_PRE, :] = jnp.concatenate(tails, axis=0).astype(BF16)

    cp_w(0, 0).wait()
    a_queries(0, [])
    cp_w(1, 1).start()
    b_block(1, retile_q(0))
    jax.lax.fori_loop(1, n_blk - 1, phase0, None)
    for cp in cp_late:
        cp.start()
    cp_w(0, n_blk - 1).wait()
    a_queries(n_blk - 1, retile_q(n_blk - 1))

    for cp in cp_late:
        cp.wait()
    for t in range(DT):
        perm_v[t, 0:D, :] = bwo_raw[:, t * LANES:(t + 1) * LANES].astype(F32)
    for t in range(DT):
        bwo_v[t] = _pack(interleaved(t, 0, range(db)))

    h_v[0:M, :] = mem0_v[...].astype(F32)
    gate = gate_v[...].astype(F32).reshape(1, D)
    a_scale = dh ** -0.5
    split = dh - LANES

    def segment(s):
        base = pl.multiple_of(s * seg, seg)
        xs = x_v[pl.ds(base, seg), :].astype(F32)
        h_v[M:L, :] = xs
        pre = pl.ds(pl.multiple_of(s * Q_PRE, Q_PRE), Q_PRE)

        lo = _iota((L, LANES), 1) < split
        zero = jnp.zeros((L, LANES), F32)
        row, col = _iota((L, 2 * L), 0), _iota((L, 2 * L), 1)
        even = col < L
        visible = (row < M) | (row >= jnp.where(even, col, col - L))

        def project(m, j):
            return [_nn(h_v[...], _unpack(w_v[m, j * PT + t])) for t in range(PT)]

        def two_heads(y):
            top = jnp.concatenate([y[0], jnp.where(lo, y[1], 0.0), zero], axis=1)
            bot = jnp.concatenate([zero, jnp.where(lo, 0.0, y[1]), y[2]], axis=1)
            return jnp.concatenate([top, bot], axis=0).astype(BF16)

        def softmax(sc):
            sc = jnp.where(visible, sc * a_scale, NEG)
            m0 = jnp.max(jnp.where(even, sc, -jnp.inf), axis=1, keepdims=True)
            m1 = jnp.max(jnp.where(even, -jnp.inf, sc), axis=1, keepdims=True)
            e = jnp.exp(sc - jnp.where(even, m0, m1))
            s0 = jnp.sum(jnp.where(even, e, 0.0), axis=1, keepdims=True)
            s1 = jnp.sum(jnp.where(even, 0.0, e), axis=1, keepdims=True)
            return e / jnp.where(even, s0, s1)

        ob = ob_v[pl.ds(base, seg), :]
        q, k, v, p, o, b, acc = {}, {}, {}, {}, {}, {}, [None] * DT
        for op, j in _schedule(n_pair, DT):
            if op == "K":
                k[j] = two_heads(project(1, j))
            elif op == "Q":
                q[j] = jnp.concatenate([
                    jnp.concatenate([_nn(h_v[0:L - Q_PRE, :], _unpack(w_v[0, c])), qpre_v[c, pre, :]], axis=0)
                    for c in range(j * PT, (j + 1) * PT)], axis=1)
            elif op == "V":
                v[j] = two_heads(project(2, j))
            elif op == "S":
                p[j] = softmax(_nt(q.pop(j), k.pop(j)))
            elif op == "P":
                o[j] = _nn(p.pop(j), v.pop(j))
            elif op == "O":
                oj = o.pop(j)
                for t in range(DT):
                    y = _nn(oj, _unpack(wo_v[t, j * dh:(j + 1) * dh, :]))
                    acc[t] = y if acc[t] is None else acc[t] + y
            else:
                b[j] = _nn(ob, _unpack(bwo_v[j]))

        g = jax.nn.sigmoid(jnp.sum(xs * gate, axis=1, keepdims=True))
        for t in range(DT):
            lanes = slice(t * LANES, (t + 1) * LANES)
            h_v[0:M, lanes] = acc[t][0:M]
            out_v[pl.ds(base, seg), lanes] = (g * acc[t][M:L] + (1.0 - g) * b[t]).astype(out_v.dtype)

    def step(i, carry):
        for u in range(UNROLL):
            segment(i * UNROLL + u)
        rows = pl.ds(pl.multiple_of(i * (UNROLL * seg), UNROLL * seg), UNROLL * seg)
        pltpu.make_async_copy(out_v.at[rows], out_hbm.at[rows], sem_out).start()
        return carry

    jax.lax.fori_loop(0, n_seg // UNROLL, step, 0)
    pltpu.make_async_copy(out_v, out_hbm, sem_out).wait()


@functools.partial(jax.jit, static_argnames=("A_seg_len",))
def pallas_gated_mix__memory_aug_recurrent_mem_tr__sliding_local_dilated__prompt_kernel(
    A_x: jax.Array,
    A_mem0: jax.Array,
    A_Wq: jax.Array,
    A_Wk: jax.Array,
    A_Wv: jax.Array,
    A_Wo: jax.Array,
    A_seg_len: int,
    B_x: jax.Array,
    B_wqkv: jax.Array,
    B_wo: jax.Array,
    gate_w: jax.Array,
):
    del B_x
    batch, S, D = A_x.shape
    _, H, dh = A_Wq.shape
    M = A_mem0.shape[1]
    E = H * dh
    seg = int(A_seg_len)
    assert batch == 1 and D % LANES == 0 and 2 * dh == 3 * LANES and H % 2 == 0
    assert S % B_BLK == 0 and S % seg == 0 and E % (S // B_BLK * LANES) == 0

    def w_t(w):
        return jnp.transpose(w, (1, 2, 0)).reshape(E, D)

    hbm = pl.BlockSpec(memory_space=pl.ANY)
    DT = D // LANES
    out = pl.pallas_call(
        functools.partial(_kernel, seg=seg, dh=dh),
        out_shape=jax.ShapeDtypeStruct((S, D), A_x.dtype),
        in_specs=[hbm] * 9,
        out_specs=hbm,
        scratch_shapes=[
            pltpu.VMEM((S, D), BF16),
            pltpu.VMEM((4, E, D), BF16),
            pltpu.VMEM((3, E // LANES, D // 2, LANES), U32),
            pltpu.VMEM((DT, E // 2, LANES), U32),
            pltpu.VMEM((D, 3 * D), BF16),
            pltpu.VMEM((D, D), BF16),
            pltpu.VMEM((3 * DT, DT, LANES // 2, LANES), U32),
            pltpu.VMEM((DT, D // 2, LANES), U32),
            pltpu.VMEM((DT, 3 * D, LANES), F32),
            pltpu.VMEM((DT, B_BLK, LANES), F32),
            pltpu.VMEM((DT, B_PAD + B_BLK, LANES), F32),
            pltpu.VMEM((DT, B_PAD + B_BLK, LANES), F32),
            pltpu.VMEM((S, D), F32),
            pltpu.VMEM((S // seg * Q_PRE, D), BF16),
            pltpu.VMEM((E // LANES, S // seg * Q_PRE, LANES), F32),
            pltpu.VMEM((M + seg, D), F32),
            pltpu.VMEM((S, D), A_x.dtype),
            pltpu.VMEM((M, D), BF16),
            pltpu.VMEM((D,), BF16),
            pltpu.SemaphoreType.DMA((6,)),
            pltpu.SemaphoreType.DMA((4, S // B_BLK)),
            pltpu.SemaphoreType.DMA(()),
        ],
        compiler_params=pltpu.CompilerParams(vmem_limit_bytes=120 * 1024 * 1024),
    )(
        A_x.reshape(S, D), A_mem0.reshape(M, D), w_t(A_Wq), w_t(A_Wk), w_t(A_Wv),
        A_Wo.reshape(E, D), B_wqkv, B_wo, gate_w,
    )
    return out.reshape(batch, S, D)
```

```python
import functools

import jax
import jax.numpy as jnp
import jax.experimental.pallas as pl
import jax.experimental.pallas.tpu as pltpu

F32 = jnp.float32
BF16 = jnp.bfloat16
U32 = jnp.uint32
LANES, SUBLANES = 128, 8
NEG = -1000000000.0

B_HEADS, B_WIN, B_DIL = 32, 8, 2
B_PAD = 16
B_BLK = 256
ORDER = (("K", 0), ("Q", 0), ("P", 2), ("V", 0), ("S", 0), ("O", 4))
B_MM = 128
SPLIT = 50
UNROLL = 4
B_EARLY = 2
Q_PRE = 8
B_SUB = 32


def _nn(a, b):
    return jax.lax.dot_general(a, b, (((1,), (0,)), ((), ())), preferred_element_type=F32)


def _nt(a, b):
    return jax.lax.dot_general(a, b, (((1,), (1,)), ((), ())), preferred_element_type=F32)


def _pack(w):
    return pltpu.bitcast(w, U32)


def _unpack(w):
    return pltpu.bitcast(w, BF16)


def _iota(shape, dim):
    return jax.lax.broadcasted_iota(jnp.int32, shape, dim)


def _interleave(main, *sides):
    for n, fn in enumerate(main):
        fn()
        for side in sides:
            for extra in side[n * len(side) // len(main):(n + 1) * len(side) // len(main)]:
                extra()


def _schedule(n_pair, n_tile):
    stages = ORDER
    ops = []
    for j in range(n_pair + max(lag for _, lag in stages)):
        ops += [(op, j - lag) for op, lag in stages if 0 <= j - lag < n_pair]
    at = ops.index(("P", n_pair - 1))
    fill = [("B", t) for t in range(n_tile)]
    return ops[:at] + fill[:B_EARLY] + ops[at:] + fill[B_EARLY:]


def _kernel(x_hbm, mem0_hbm, wq_hbm, wk_hbm, wv_hbm, wo_hbm, bqkv_hbm, bwo_hbm, gate_hbm,
            out_hbm,
            x_v, stage, w_v, wo_v, bqkv_raw, bwo_raw, bqkv_v, bwo_v, perm_v, qb_v, kb_v, vb_v, ob_v,
            xpre_v, qpre_v, h_v, out_v, mem0_v, gate_v, sem_in, sem_w, sem_out, *, seg, dh):
    S, D = x_v.shape
    M = mem0_v.shape[0]
    L = M + seg
    E = stage.shape[1]
    DT = D // LANES
    PT = 2 * dh // LANES
    n_pair = E // (2 * dh)
    n_seg = S // seg
    n_blk = S // B_BLK
    q_tiles = E // LANES // n_blk
    r_tiles = E // LANES // (n_blk - 2)
    w_hbm = (wq_hbm, wk_hbm, wv_hbm, wo_hbm)

    cp_bqkv = pltpu.make_async_copy(bqkv_hbm, bqkv_raw, sem_in.at[0])
    head, tail = pl.ds(0, B_BLK), pl.ds(B_BLK, S - B_BLK)
    cp_x0 = pltpu.make_async_copy(x_hbm.at[head], x_v.at[head], sem_in.at[1])
    cp_x1 = pltpu.make_async_copy(x_hbm.at[tail], x_v.at[tail], sem_in.at[2])
    cp_late = [pltpu.make_async_copy(src, dst, sem_in.at[3 + n])
               for n, (src, dst) in enumerate(((bwo_hbm, bwo_raw), (mem0_hbm, mem0_v), (gate_hbm, gate_v)))]

    def cp_w(m, c):
        n = (r_tiles if m else q_tiles) * LANES
        rows = pl.ds(c * n, n)
        return pltpu.make_async_copy(w_hbm[m].at[rows], stage.at[m, rows], sem_w.at[m, c])

    cp_bqkv.start()
    cp_x0.start()
    cp_x0.wait()
    cp_bqkv.wait()
    cp_x1.start()
    cp_w(0, 0).start()

    db = D // B_HEADS

    def interleaved(t, first, ds):
        return jnp.concatenate(
            [perm_v[t, pl.ds(first + d, B_HEADS, stride=db), :] for d in ds], axis=0).astype(BF16)

    def b_transpose(c):
        wt = bqkv_raw[:, c * LANES:(c + 1) * LANES].T.astype(F32)
        for t in range(DT):
            perm_v[t, c * LANES:(c + 1) * LANES, :] = wt[:, t * LANES:(t + 1) * LANES]

    def b_gather(c):
        per_tile = LANES // B_HEADS
        ds = range(c % DT * per_tile, (c % DT + 1) * per_tile)
        for t in range(DT):
            bqkv_v[c, t] = _pack(interleaved(t, c // DT * D, ds))

    def b_project(xb, c):
        return _nt(xb, jnp.concatenate([_unpack(bqkv_v[c, t]) for t in range(DT)], axis=1))

    b_scale = db ** -0.5

    def window_attention(base, r):
        q = [qb_v[t, r:r + B_SUB, :] for t in range(DT)]
        pos = base + r + _iota((B_SUB, LANES), 0)

        rows = [slice(r + B_PAD - w * B_DIL, r + B_PAD - w * B_DIL + B_SUB) for w in range(B_WIN)]
        logits = []
        for w in range(B_WIN):
            acc = functools.reduce(jnp.add, [q[t] * kb_v[t, rows[w], :] for t in range(DT)])
            shift = LANES // 2
            while shift >= B_HEADS:
                acc = acc + pltpu.roll(acc, shift, 1)
                shift //= 2
            acc = acc * b_scale
            logits.append(jnp.where(pos >= w * B_DIL, acc, NEG) if w else acc)
        mx = functools.reduce(jnp.maximum, logits)
        ex = [jnp.exp(l - mx) for l in logits]
        inv = 1.0 / functools.reduce(jnp.add, ex)
        for t in range(DT):
            acc = functools.reduce(jnp.add, [ex[w] * vb_v[t, rows[w], :] for w in range(B_WIN)])
            ob_v[pl.ds(pl.multiple_of(base + r, B_SUB), B_SUB), t * LANES:(t + 1) * LANES] = acc * inv

    task = functools.partial

    def b_qkv(blk, r, c):
        y = b_project(x_v[pl.ds(pl.multiple_of(blk * B_BLK + r, B_MM), B_MM), :], c)
        if c < DT:
            qb_v[c, r:r + B_MM, :] = y
        else:
            (kb_v, vb_v)[c // DT - 1][c % DT, B_PAD + r:B_PAD + r + B_MM, :] = y

    def b_attend(blk, r):
        return [task(window_attention, blk * B_BLK, r + u) for u in range(0, B_MM, B_SUB)]

    def b_block(blk, side, first=False):
        for r in range(0, B_BLK, B_MM):
            _interleave([task(b_qkv, blk, r, c) for c in range(3 * DT)], side)
            if first and r == 0:
                kb_v[:, 0:B_PAD, :] = jnp.zeros((DT, B_PAD, LANES), F32)
                for t in range(DT):
                    vb_v[t, 0:B_PAD, :] = jnp.broadcast_to(vb_v[t, B_PAD:B_PAD + 1, :], (B_PAD, LANES))
            side = b_attend(blk, r)

    def slab(tile):
        return pl.ds(pl.multiple_of(tile * LANES, LANES), LANES)

    def a_queries(i, side):
        def one(r, tile):
            qpre_v[tile, r:r + B_MM, :] = _nt(xpre_v[r:r + B_MM, :], stage[0, slab(tile), :])

        _interleave([task(one, r, i * q_tiles + k) for k in range(q_tiles)
                     for r in range(0, n_seg * Q_PRE, B_MM)], b_attend(i, B_BLK - B_MM), side)
        for ref in (kb_v, vb_v):
            ref[:, 0:B_PAD, :] = ref[:, B_BLK:B_BLK + B_PAD, :]

    def retile(m, tile, t, src=None):
        src_m, src_tile = src or (m, tile)
        w = stage[src_m, slab(src_tile), t * LANES:(t + 1) * LANES]
        if m < 3:
            w_v[m, tile, t * LANES // 2:(t + 1) * LANES // 2, :] = _pack(w.T)
        else:
            wo_v[t, pl.ds(pl.multiple_of(tile * (LANES // 2), LANES // 2), LANES // 2), :] = _pack(w)

    def retile_q(i):
        return [task(retile, 0, i * q_tiles + k, t) for k in range(q_tiles) for t in range(DT)]

    def phase0(i, carry):
        @pl.when(i > 0)
        def _():
            cp_w(0, i + 1).start()

        @pl.when(i + 2 < n_blk)
        def _():
            cp_w(2, i).start()
            cp_w(3, i).start()

        @pl.when(i + 3 < n_blk)
        def _():
            cp_w(1, i + 1).start()

        cp_w(0, i).wait()

        @pl.when(i > 0)
        def _():
            for m in range(1, 4):
                cp_w(m, i - 1).wait()

        side = retile_q(i)
        later = jnp.minimum(i, 1)
        for k in range(r_tiles):
            tile = (i - later) * r_tiles + k
            side += [task(retile, m, tile, t, (m * later, tile * later)) for t in range(DT) for m in range(1, 4)]
        n = len(side) * SPLIT // 100
        a_queries(i, side[:n])
        b_block(i + 1, side[n:])

    prep = [task(fn, m * DT + t) for m in range(3) for fn in (b_transpose, b_gather) for t in range(DT)]
    for fn in prep[:2 * DT]:
        fn()
    cp_w(0, 1).start()
    b_block(0, prep[2 * DT:] + [lambda: None] * (2 * DT), first=True)
    cp_w(1, 0).start()
    cp_x1.wait()

    for s in range(0, n_seg, 2):
        tails = [x_v[e - 2 * Q_PRE:e, :].astype(F32)[Q_PRE:] for e in ((s + 1) * seg, (s + 2) * seg)]
        xpre_v[s * Q_PRE:(s + 2) * Q_PRE, :] = jnp.concatenate(tails, axis=0).astype(BF16)

    jax.lax.fori_loop(0, n_blk - 1, phase0, None)
    for cp in cp_late:
        cp.start()
    cp_w(0, n_blk - 1).wait()
    a_queries(n_blk - 1, retile_q(n_blk - 1))

    for cp in cp_late:
        cp.wait()
    for t in range(DT):
        perm_v[t, 0:D, :] = bwo_raw[:, t * LANES:(t + 1) * LANES].astype(F32)
    for t in range(DT):
        bwo_v[t] = _pack(interleaved(t, 0, range(db)))

    h_v[0:M, :] = mem0_v[...].astype(F32)
    gate = gate_v[...].astype(F32).reshape(1, D)
    a_scale = dh ** -0.5
    split = dh - LANES

    def segment(s):
        base = pl.multiple_of(s * seg, seg)
        xs = x_v[pl.ds(base, seg), :].astype(F32)
        h_v[M:L, :] = xs
        pre = pl.ds(pl.multiple_of(s * Q_PRE, Q_PRE), Q_PRE)

        lo = _iota((L, LANES), 1) < split
        zero = jnp.zeros((L, LANES), F32)
        row, col = _iota((L, 2 * L), 0), _iota((L, 2 * L), 1)
        even = col < L
        visible = (row < M) | (row >= jnp.where(even, col, col - L))

        def project(m, j):
            return [_nn(h_v[...], _unpack(w_v[m, j * PT + t])) for t in range(PT)]

        def two_heads(y):
            top = jnp.concatenate([y[0], jnp.where(lo, y[1], 0.0), zero], axis=1)
            bot = jnp.concatenate([zero, jnp.where(lo, 0.0, y[1]), y[2]], axis=1)
            return jnp.concatenate([top, bot], axis=0).astype(BF16)

        def softmax(sc):
            sc = jnp.where(visible, sc * a_scale, NEG)
            m0 = jnp.max(jnp.where(even, sc, -jnp.inf), axis=1, keepdims=True)
            m1 = jnp.max(jnp.where(even, -jnp.inf, sc), axis=1, keepdims=True)
            e = jnp.exp(sc - jnp.where(even, m0, m1))
            s0 = jnp.sum(jnp.where(even, e, 0.0), axis=1, keepdims=True)
            s1 = jnp.sum(jnp.where(even, 0.0, e), axis=1, keepdims=True)
            return e / jnp.where(even, s0, s1)

        ob = ob_v[pl.ds(base, seg), :]
        q, k, v, p, o, b, acc = {}, {}, {}, {}, {}, {}, [None] * DT
        for op, j in _schedule(n_pair, DT):
            if op == "K":
                k[j] = two_heads(project(1, j))
            elif op == "Q":
                q[j] = jnp.concatenate([
                    jnp.concatenate([_nn(h_v[0:L - Q_PRE, :], _unpack(w_v[0, c])), qpre_v[c, pre, :]], axis=0)
                    for c in range(j * PT, (j + 1) * PT)], axis=1)
            elif op == "V":
                v[j] = two_heads(project(2, j))
            elif op == "S":
                p[j] = softmax(_nt(q.pop(j), k.pop(j)))
            elif op == "P":
                o[j] = _nn(p.pop(j), v.pop(j))
            elif op == "O":
                oj = o.pop(j)
                for t in range(DT):
                    y = _nn(oj, _unpack(wo_v[t, j * dh:(j + 1) * dh, :]))
                    acc[t] = y if acc[t] is None else acc[t] + y
            else:
                b[j] = _nn(ob, _unpack(bwo_v[j]))

        g = jax.nn.sigmoid(jnp.sum(xs * gate, axis=1, keepdims=True))
        for t in range(DT):
            lanes = slice(t * LANES, (t + 1) * LANES)
            h_v[0:M, lanes] = acc[t][0:M]
            out_v[pl.ds(base, seg), lanes] = (g * acc[t][M:L] + (1.0 - g) * b[t]).astype(out_v.dtype)

    def step(i, carry):
        for u in range(UNROLL):
            segment(i * UNROLL + u)
        rows = pl.ds(pl.multiple_of(i * (UNROLL * seg), UNROLL * seg), UNROLL * seg)
        pltpu.make_async_copy(out_v.at[rows], out_hbm.at[rows], sem_out).start()
        return carry

    jax.lax.fori_loop(0, n_seg // UNROLL, step, 0)
    pltpu.make_async_copy(out_v, out_hbm, sem_out).wait()


@functools.partial(jax.jit, static_argnames=("A_seg_len",))
def pallas_gated_mix__memory_aug_recurrent_mem_tr__sliding_local_dilated__prompt_kernel(
    A_x: jax.Array,
    A_mem0: jax.Array,
    A_Wq: jax.Array,
    A_Wk: jax.Array,
    A_Wv: jax.Array,
    A_Wo: jax.Array,
    A_seg_len: int,
    B_x: jax.Array,
    B_wqkv: jax.Array,
    B_wo: jax.Array,
    gate_w: jax.Array,
):
    del B_x
    batch, S, D = A_x.shape
    _, H, dh = A_Wq.shape
    M = A_mem0.shape[1]
    E = H * dh
    seg = int(A_seg_len)
    assert batch == 1 and D % LANES == 0 and 2 * dh == 3 * LANES and H % 2 == 0
    assert S % B_BLK == 0 and S % seg == 0 and E % (S // B_BLK * LANES) == 0

    def w_t(w):
        return jnp.transpose(w, (1, 2, 0)).reshape(E, D)

    hbm = pl.BlockSpec(memory_space=pl.ANY)
    DT = D // LANES
    out = pl.pallas_call(
        functools.partial(_kernel, seg=seg, dh=dh),
        out_shape=jax.ShapeDtypeStruct((S, D), A_x.dtype),
        in_specs=[hbm] * 9,
        out_specs=hbm,
        scratch_shapes=[
            pltpu.VMEM((S, D), BF16),
            pltpu.VMEM((4, E, D), BF16),
            pltpu.VMEM((3, E // LANES, D // 2, LANES), U32),
            pltpu.VMEM((DT, E // 2, LANES), U32),
            pltpu.VMEM((D, 3 * D), BF16),
            pltpu.VMEM((D, D), BF16),
            pltpu.VMEM((3 * DT, DT, LANES // 2, LANES), U32),
            pltpu.VMEM((DT, D // 2, LANES), U32),
            pltpu.VMEM((DT, 3 * D, LANES), F32),
            pltpu.VMEM((DT, B_BLK, LANES), F32),
            pltpu.VMEM((DT, B_PAD + B_BLK, LANES), F32),
            pltpu.VMEM((DT, B_PAD + B_BLK, LANES), F32),
            pltpu.VMEM((S, D), F32),
            pltpu.VMEM((S // seg * Q_PRE, D), BF16),
            pltpu.VMEM((E // LANES, S // seg * Q_PRE, LANES), F32),
            pltpu.VMEM((M + seg, D), F32),
            pltpu.VMEM((S, D), A_x.dtype),
            pltpu.VMEM((M, D), BF16),
            pltpu.VMEM((D,), BF16),
            pltpu.SemaphoreType.DMA((6,)),
            pltpu.SemaphoreType.DMA((4, S // B_BLK)),
            pltpu.SemaphoreType.DMA(()),
        ],
        compiler_params=pltpu.CompilerParams(vmem_limit_bytes=120 * 1024 * 1024),
    )(
        A_x.reshape(S, D), A_mem0.reshape(M, D), w_t(A_Wq), w_t(A_Wk), w_t(A_Wv),
        A_Wo.reshape(E, D), B_wqkv, B_wo, gate_w,
    )
    return out.reshape(batch, S, D)
```

```python
import functools

import jax
import jax.numpy as jnp
import jax.experimental.pallas as pl
import jax.experimental.pallas.tpu as pltpu

F32 = jnp.float32
BF16 = jnp.bfloat16
U32 = jnp.uint32
LANES, SUBLANES = 128, 8
NEG = -1000000000.0

B_HEADS, B_WIN, B_DIL = 32, 8, 2
B_PAD = 16
B_BLK = 256
ORDER = (("K", 0), ("Q", 0), ("P", 2), ("V", 0), ("S", 0), ("O", 4))
B_MM = 128
SPLIT = 50
UNROLL = 4
B_EARLY = 2
Q_PRE = 8
B_SUB = 32


def _nn(a, b):
    return jax.lax.dot_general(a, b, (((1,), (0,)), ((), ())), preferred_element_type=F32)


def _nt(a, b):
    return jax.lax.dot_general(a, b, (((1,), (1,)), ((), ())), preferred_element_type=F32)


def _pack(w):
    return pltpu.bitcast(w, U32)


def _unpack(w):
    return pltpu.bitcast(w, BF16)


def _iota(shape, dim):
    return jax.lax.broadcasted_iota(jnp.int32, shape, dim)


def _interleave(main, *sides):
    for n, fn in enumerate(main):
        fn()
        for side in sides:
            for extra in side[n * len(side) // len(main):(n + 1) * len(side) // len(main)]:
                extra()


def _schedule(n_pair, n_tile):
    stages = ORDER
    ops = []
    for j in range(n_pair + max(lag for _, lag in stages)):
        ops += [(op, j - lag) for op, lag in stages if 0 <= j - lag < n_pair]
    at = ops.index(("P", n_pair - 1))
    fill = [("B", t) for t in range(n_tile)]
    return ops[:at] + fill[:B_EARLY] + ops[at:] + fill[B_EARLY:]


def _kernel(x_hbm, mem0_hbm, wq_hbm, wk_hbm, wv_hbm, wo_hbm, bqkv_hbm, bwo_hbm, gate_hbm,
            out_hbm,
            x_v, stage, w_v, wo_v, bqkv_raw, bwo_raw, bqkv_v, bwo_v, perm_v, qb_v, kb_v, vb_v, ob_v,
            xpre_v, qpre_v, h_v, out_v, mem0_v, gate_v, sem_in, sem_w, sem_out, *, seg, dh):
    S, D = x_v.shape
    M = mem0_v.shape[0]
    L = M + seg
    E = stage.shape[1]
    DT = D // LANES
    PT = 2 * dh // LANES
    n_pair = E // (2 * dh)
    n_seg = S // seg
    n_blk = S // B_BLK
    q_tiles = E // LANES // n_blk
    r_tiles = E // LANES // (n_blk - 2)
    w_hbm = (wq_hbm, wk_hbm, wv_hbm, wo_hbm)

    cp_bqkv = pltpu.make_async_copy(bqkv_hbm, bqkv_raw, sem_in.at[0])
    head, tail = pl.ds(0, B_BLK), pl.ds(B_BLK, S - B_BLK)
    cp_x0 = pltpu.make_async_copy(x_hbm.at[head], x_v.at[head], sem_in.at[1])
    cp_x1 = pltpu.make_async_copy(x_hbm.at[tail], x_v.at[tail], sem_in.at[2])
    cp_late = [pltpu.make_async_copy(src, dst, sem_in.at[3 + n])
               for n, (src, dst) in enumerate(((bwo_hbm, bwo_raw), (mem0_hbm, mem0_v), (gate_hbm, gate_v)))]

    def cp_w(m, c):
        n = (r_tiles if m else q_tiles) * LANES
        rows = pl.ds(c * n, n)
        return pltpu.make_async_copy(w_hbm[m].at[rows], stage.at[m, rows], sem_w.at[m, c])

    cp_bqkv.start()
    cp_x0.start()
    cp_x0.wait()
    cp_bqkv.wait()
    cp_x1.start()
    cp_w(0, 0).start()

    db = D // B_HEADS

    def interleaved(t, first, ds):
        return jnp.concatenate(
            [perm_v[t, pl.ds(first + d, B_HEADS, stride=db), :] for d in ds], axis=0).astype(BF16)

    def b_transpose(c):
        wt = bqkv_raw[:, c * LANES:(c + 1) * LANES].T.astype(F32)
        for t in range(DT):
            perm_v[t, c * LANES:(c + 1) * LANES, :] = wt[:, t * LANES:(t + 1) * LANES]

    def b_gather(c):
        per_tile = LANES // B_HEADS
        ds = range(c % DT * per_tile, (c % DT + 1) * per_tile)
        for t in range(DT):
            bqkv_v[c, t] = _pack(interleaved(t, c // DT * D, ds))

    def b_project(xb, c):
        return _nt(xb, jnp.concatenate([_unpack(bqkv_v[c, t]) for t in range(DT)], axis=1))

    b_scale = db ** -0.5

    def window_attention(base, r):
        q = [qb_v[t, r:r + B_SUB, :] for t in range(DT)]
        pos = base + r + _iota((B_SUB, LANES), 0)

        rows = [slice(r + B_PAD - w * B_DIL, r + B_PAD - w * B_DIL + B_SUB) for w in range(B_WIN)]
        logits = []
        for w in range(B_WIN):
            acc = functools.reduce(jnp.add, [q[t] * kb_v[t, rows[w], :] for t in range(DT)])
            shift = LANES // 2
            while shift >= B_HEADS:
                acc = acc + pltpu.roll(acc, shift, 1)
                shift //= 2
            acc = acc * b_scale
            logits.append(jnp.where(pos >= w * B_DIL, acc, NEG) if w else acc)
        mx = functools.reduce(jnp.maximum, logits)
        ex = [jnp.exp(l - mx) for l in logits]
        inv = 1.0 / functools.reduce(jnp.add, ex)
        for t in range(DT):
            acc = functools.reduce(jnp.add, [ex[w] * vb_v[t, rows[w], :] for w in range(B_WIN)])
            ob_v[pl.ds(pl.multiple_of(base + r, B_SUB), B_SUB), t * LANES:(t + 1) * LANES] = acc * inv

    task = functools.partial

    def b_qkv(blk, r, c):
        y = b_project(x_v[pl.ds(pl.multiple_of(blk * B_BLK + r, B_MM), B_MM), :], c)
        if c < DT:
            qb_v[c, r:r + B_MM, :] = y
        else:
            (kb_v, vb_v)[c // DT - 1][c % DT, B_PAD + r:B_PAD + r + B_MM, :] = y

    def b_attend(blk, r):
        return [task(window_attention, blk * B_BLK, r + u) for u in range(0, B_MM, B_SUB)]

    def b_block(blk, side, first=False):
        for r in range(0, B_BLK, B_MM):
            _interleave([task(b_qkv, blk, r, c) for c in range(3 * DT)], side)
            if first and r == 0:
                kb_v[:, 0:B_PAD, :] = jnp.zeros((DT, B_PAD, LANES), F32)
                for t in range(DT):
                    vb_v[t, 0:B_PAD, :] = jnp.broadcast_to(vb_v[t, B_PAD:B_PAD + 1, :], (B_PAD, LANES))
            side = b_attend(blk, r)

    def slab(tile):
        return pl.ds(pl.multiple_of(tile * LANES, LANES), LANES)

    def a_queries(i, side):
        def one(r, tile):
            qpre_v[tile, r:r + B_MM, :] = _nt(xpre_v[r:r + B_MM, :], stage[0, slab(tile), :])

        _interleave([task(one, r, i * q_tiles + k) for k in range(q_tiles)
                     for r in range(0, n_seg * Q_PRE, B_MM)], b_attend(i, B_BLK - B_MM), side)
        for ref in (kb_v, vb_v):
            ref[:, 0:B_PAD, :] = ref[:, B_BLK:B_BLK + B_PAD, :]

    def retile(m, tile, t, src=None):
        src_m, src_tile = src or (m, tile)
        w = stage[src_m, slab(src_tile), t * LANES:(t + 1) * LANES]
        if m < 3:
            w_v[m, tile, t * LANES // 2:(t + 1) * LANES // 2, :] = _pack(w.T)
        else:
            wo_v[t, pl.ds(pl.multiple_of(tile * (LANES // 2), LANES // 2), LANES // 2), :] = _pack(w)

    def retile_q(i):
        return [task(retile, 0, i * q_tiles + k, t) for k in range(q_tiles) for t in range(DT)]

    def phase0(i, carry):
        @pl.when(i > 0)
        def _():
            cp_w(0, i + 1).start()

        @pl.when(i + 2 < n_blk)
        def _():
            cp_w(2, i).start()
            cp_w(3, i).start()

        @pl.when(i + 3 < n_blk)
        def _():
            cp_w(1, i + 1).start()

        @pl.when(i + 2 == n_blk)
        def _():
            for cp in cp_late:
                cp.start()

        cp_w(0, i).wait()

        @pl.when(i > 0)
        def _():
            for m in range(1, 4):
                cp_w(m, i - 1).wait()

        side = retile_q(i)
        later = jnp.minimum(i, 1)
        for k in range(r_tiles):
            tile = (i - later) * r_tiles + k
            side += [task(retile, m, tile, t, (m * later, tile * later)) for t in range(DT) for m in range(1, 4)]
        n = len(side) * SPLIT // 100
        a_queries(i, side[:n])
        b_block(i + 1, side[n:])

    prep = [task(fn, m * DT + t) for m in range(3) for fn in (b_transpose, b_gather) for t in range(DT)]
    for fn in prep[:2 * DT]:
        fn()
    cp_w(0, 1).start()
    b_block(0, prep[2 * DT:] + [lambda: None] * (2 * DT), first=True)
    cp_w(1, 0).start()
    cp_x1.wait()

    for s in range(0, n_seg, 2):
        tails = [x_v[e - 2 * Q_PRE:e, :].astype(F32)[Q_PRE:] for e in ((s + 1) * seg, (s + 2) * seg)]
        xpre_v[s * Q_PRE:(s + 2) * Q_PRE, :] = jnp.concatenate(tails, axis=0).astype(BF16)

    jax.lax.fori_loop(0, n_blk - 1, phase0, None)
    cp_w(0, n_blk - 1).wait()
    for cp in cp_late:
        cp.wait()

    def b_out_weights(t):
        perm_v[t, 0:D, :] = bwo_raw[:, t * LANES:(t + 1) * LANES].astype(F32)
        bwo_v[t] = _pack(interleaved(t, 0, range(db)))

    a_queries(n_blk - 1, retile_q(n_blk - 1) + [task(b_out_weights, t) for t in range(DT)])

    h_v[0:M, :] = mem0_v[...].astype(F32)
    gate = gate_v[...].astype(F32).reshape(1, D)
    a_scale = dh ** -0.5
    split = dh - LANES

    def segment(s):
        base = pl.multiple_of(s * seg, seg)
        xs = x_v[pl.ds(base, seg), :].astype(F32)
        h_v[M:L, :] = xs
        pre = pl.ds(pl.multiple_of(s * Q_PRE, Q_PRE), Q_PRE)

        lo = _iota((L, LANES), 1) < split
        zero = jnp.zeros((L, LANES), F32)
        row, col = _iota((L, 2 * L), 0), _iota((L, 2 * L), 1)
        even = col < L
        visible = (row < M) | (row >= jnp.where(even, col, col - L))

        def project(m, j):
            return [_nn(h_v[...], _unpack(w_v[m, j * PT + t])) for t in range(PT)]

        def two_heads(y):
            top = jnp.concatenate([y[0], jnp.where(lo, y[1], 0.0), zero], axis=1)
            bot = jnp.concatenate([zero, jnp.where(lo, 0.0, y[1]), y[2]], axis=1)
            return jnp.concatenate([top, bot], axis=0).astype(BF16)

        def softmax(sc):
            sc = jnp.where(visible, sc * a_scale, NEG)
            m0 = jnp.max(jnp.where(even, sc, -jnp.inf), axis=1, keepdims=True)
            m1 = jnp.max(jnp.where(even, -jnp.inf, sc), axis=1, keepdims=True)
            e = jnp.exp(sc - jnp.where(even, m0, m1))
            s0 = jnp.sum(jnp.where(even, e, 0.0), axis=1, keepdims=True)
            s1 = jnp.sum(jnp.where(even, 0.0, e), axis=1, keepdims=True)
            return e / jnp.where(even, s0, s1)

        ob = ob_v[pl.ds(base, seg), :]
        q, k, v, p, o, b, acc = {}, {}, {}, {}, {}, {}, [None] * DT
        for op, j in _schedule(n_pair, DT):
            if op == "K":
                k[j] = two_heads(project(1, j))
            elif op == "Q":
                q[j] = jnp.concatenate([
                    jnp.concatenate([_nn(h_v[0:L - Q_PRE, :], _unpack(w_v[0, c])), qpre_v[c, pre, :]], axis=0)
                    for c in range(j * PT, (j + 1) * PT)], axis=1)
            elif op == "V":
                v[j] = two_heads(project(2, j))
            elif op == "S":
                p[j] = softmax(_nt(q.pop(j), k.pop(j)))
            elif op == "P":
                o[j] = _nn(p.pop(j), v.pop(j))
            elif op == "O":
                oj = o.pop(j)
                for t in range(DT):
                    y = _nn(oj, _unpack(wo_v[t, j * dh:(j + 1) * dh, :]))
                    acc[t] = y if acc[t] is None else acc[t] + y
            else:
                b[j] = _nn(ob, _unpack(bwo_v[j]))

        g = jax.nn.sigmoid(jnp.sum(xs * gate, axis=1, keepdims=True))
        for t in range(DT):
            lanes = slice(t * LANES, (t + 1) * LANES)
            h_v[0:M, lanes] = acc[t][0:M]
            out_v[pl.ds(base, seg), lanes] = (g * acc[t][M:L] + (1.0 - g) * b[t]).astype(out_v.dtype)

    def step(i, carry):
        for u in range(UNROLL):
            segment(i * UNROLL + u)
        rows = pl.ds(pl.multiple_of(i * (UNROLL * seg), UNROLL * seg), UNROLL * seg)
        pltpu.make_async_copy(out_v.at[rows], out_hbm.at[rows], sem_out).start()
        return carry

    jax.lax.fori_loop(0, n_seg // UNROLL, step, 0)
    pltpu.make_async_copy(out_v, out_hbm, sem_out).wait()


@functools.partial(jax.jit, static_argnames=("A_seg_len",))
def pallas_gated_mix__memory_aug_recurrent_mem_tr__sliding_local_dilated__prompt_kernel(
    A_x: jax.Array,
    A_mem0: jax.Array,
    A_Wq: jax.Array,
    A_Wk: jax.Array,
    A_Wv: jax.Array,
    A_Wo: jax.Array,
    A_seg_len: int,
    B_x: jax.Array,
    B_wqkv: jax.Array,
    B_wo: jax.Array,
    gate_w: jax.Array,
):
    del B_x
    batch, S, D = A_x.shape
    _, H, dh = A_Wq.shape
    M = A_mem0.shape[1]
    E = H * dh
    seg = int(A_seg_len)
    assert batch == 1 and D % LANES == 0 and 2 * dh == 3 * LANES and H % 2 == 0
    assert S % B_BLK == 0 and S % seg == 0 and E % (S // B_BLK * LANES) == 0

    def w_t(w):
        return jnp.transpose(w, (1, 2, 0)).reshape(E, D)

    hbm = pl.BlockSpec(memory_space=pl.ANY)
    DT = D // LANES
    out = pl.pallas_call(
        functools.partial(_kernel, seg=seg, dh=dh),
        out_shape=jax.ShapeDtypeStruct((S, D), A_x.dtype),
        in_specs=[hbm] * 9,
        out_specs=hbm,
        scratch_shapes=[
            pltpu.VMEM((S, D), BF16),
            pltpu.VMEM((4, E, D), BF16),
            pltpu.VMEM((3, E // LANES, D // 2, LANES), U32),
            pltpu.VMEM((DT, E // 2, LANES), U32),
            pltpu.VMEM((D, 3 * D), BF16),
            pltpu.VMEM((D, D), BF16),
            pltpu.VMEM((3 * DT, DT, LANES // 2, LANES), U32),
            pltpu.VMEM((DT, D // 2, LANES), U32),
            pltpu.VMEM((DT, 3 * D, LANES), F32),
            pltpu.VMEM((DT, B_BLK, LANES), F32),
            pltpu.VMEM((DT, B_PAD + B_BLK, LANES), F32),
            pltpu.VMEM((DT, B_PAD + B_BLK, LANES), F32),
            pltpu.VMEM((S, D), F32),
            pltpu.VMEM((S // seg * Q_PRE, D), BF16),
            pltpu.VMEM((E // LANES, S // seg * Q_PRE, LANES), F32),
            pltpu.VMEM((M + seg, D), F32),
            pltpu.VMEM((S, D), A_x.dtype),
            pltpu.VMEM((M, D), BF16),
            pltpu.VMEM((D,), BF16),
            pltpu.SemaphoreType.DMA((6,)),
            pltpu.SemaphoreType.DMA((4, S // B_BLK)),
            pltpu.SemaphoreType.DMA(()),
        ],
        compiler_params=pltpu.CompilerParams(vmem_limit_bytes=120 * 1024 * 1024),
    )(
        A_x.reshape(S, D), A_mem0.reshape(M, D), w_t(A_Wq), w_t(A_Wk), w_t(A_Wv),
        A_Wo.reshape(E, D), B_wqkv, B_wo, gate_w,
    )
    return out.reshape(batch, S, D)
```

```python
import functools

import jax
import jax.numpy as jnp
import jax.experimental.pallas as pl
import jax.experimental.pallas.tpu as pltpu

F32 = jnp.float32
BF16 = jnp.bfloat16
U32 = jnp.uint32
LANES, SUBLANES = 128, 8
NEG = -1000000000.0

B_HEADS, B_WIN, B_DIL = 32, 8, 2
B_PAD = 16
B_BLK = 256
ORDER = (("K", 0), ("Q", 0), ("P", 2), ("V", 0), ("S", 0), ("O", 4))
B_MM = 128
SPLIT = 50
UNROLL = 4
W_AT = 30
B_EARLY = 2
Q_PRE = 8
B_SUB = 32


def _nn(a, b):
    return jax.lax.dot_general(a, b, (((1,), (0,)), ((), ())), preferred_element_type=F32)


def _nt(a, b):
    return jax.lax.dot_general(a, b, (((1,), (1,)), ((), ())), preferred_element_type=F32)


def _pack(w):
    return pltpu.bitcast(w, U32)


def _unpack(w):
    return pltpu.bitcast(w, BF16)


def _iota(shape, dim):
    return jax.lax.broadcasted_iota(jnp.int32, shape, dim)


def _interleave(main, *sides):
    for n, fn in enumerate(main):
        fn()
        for side in sides:
            for extra in side[n * len(side) // len(main):(n + 1) * len(side) // len(main)]:
                extra()


def _schedule(n_pair, n_tile):
    stages = ORDER
    ops = []
    for j in range(n_pair + max(lag for _, lag in stages)):
        ops += [(op, j - lag) for op, lag in stages if 0 <= j - lag < n_pair]
    at = ops.index(("P", n_pair - 1))
    fill = [("B", t) for t in range(n_tile)]
    ops = ops[:W_AT] + [("W", 0)] + ops[W_AT:]
    at += 1
    return ops[:at] + fill[:B_EARLY] + ops[at:] + fill[B_EARLY:]


def _kernel(x_hbm, mem0_hbm, wq_hbm, wk_hbm, wv_hbm, wo_hbm, bqkv_hbm, bwo_hbm, gate_hbm,
            out_hbm,
            x_v, stage, w_v, wo_v, bqkv_raw, bwo_raw, bqkv_v, bwo_v, perm_v, qkv_v,
            xpre_v, qpre_v, h_v, out_v, mem0_v, gate_v, sem_in, sem_w, sem_out, *, seg, dh):
    S, D = x_v.shape
    M = mem0_v.shape[0]
    L = M + seg
    E = stage.shape[1]
    DT = D // LANES
    PT = 2 * dh // LANES
    n_pair = E // (2 * dh)
    n_seg = S // seg
    n_blk = S // B_BLK
    q_tiles = E // LANES // n_blk
    r_tiles = pl.cdiv(E // LANES, n_blk - 1)
    r_last = E // LANES - (n_blk - 2) * r_tiles
    w_hbm = (wq_hbm, wk_hbm, wv_hbm, wo_hbm)

    cp_bqkv = pltpu.make_async_copy(bqkv_hbm, bqkv_raw, sem_in.at[0])
    head, tail = pl.ds(0, B_BLK), pl.ds(B_BLK, S - B_BLK)
    cp_x0 = pltpu.make_async_copy(x_hbm.at[head], x_v.at[head], sem_in.at[1])
    cp_x1 = pltpu.make_async_copy(x_hbm.at[tail], x_v.at[tail], sem_in.at[2])
    cp_late = [pltpu.make_async_copy(src, dst, sem_in.at[3 + n])
               for n, (src, dst) in enumerate(((bwo_hbm, bwo_raw), (mem0_hbm, mem0_v), (gate_hbm, gate_v)))]

    def cp_w(m, c, last=False):
        n = (r_tiles if m else q_tiles) * LANES
        rows = pl.ds(c * n, r_last * LANES if last else n)
        return pltpu.make_async_copy(w_hbm[m].at[rows], stage.at[m, rows], sem_w.at[m, c])

    cp_bqkv.start()
    cp_x0.start()
    cp_x0.wait()
    cp_bqkv.wait()
    cp_x1.start()
    cp_w(0, 0).start()

    db = D // B_HEADS

    def interleaved(t, first, ds):
        return jnp.concatenate(
            [perm_v[t, pl.ds(first + d, B_HEADS, stride=db), :] for d in ds], axis=0).astype(BF16)

    def b_transpose(c):
        wt = bqkv_raw[:, c * LANES:(c + 1) * LANES].T.astype(F32)
        for t in range(DT):
            perm_v[t, c * LANES:(c + 1) * LANES, :] = wt[:, t * LANES:(t + 1) * LANES]

    def b_gather(c):
        per_tile = LANES // B_HEADS
        ds = range(c % DT * per_tile, (c % DT + 1) * per_tile)
        for t in range(DT):
            bqkv_v[c, t] = _pack(interleaved(t, c // DT * D, ds))

    def b_project(xb, c):
        return _nt(xb, jnp.concatenate([_unpack(bqkv_v[c, t]) for t in range(DT)], axis=1))

    b_scale = db ** -0.5

    def window_attention(base):
        q = [qkv_v[t, pl.ds(base + B_PAD, seg), :] for t in range(DT)]
        pos = base + _iota((seg, LANES), 0)

        rows = [pl.ds(base + (B_PAD - w * B_DIL), seg) for w in range(B_WIN)]
        logits = []
        for w in range(B_WIN):
            acc = functools.reduce(jnp.add, [q[t] * qkv_v[DT + t, rows[w], :] for t in range(DT)])
            shift = LANES // 2
            while shift >= B_HEADS:
                acc = acc + pltpu.roll(acc, shift, 1)
                shift //= 2
            acc = acc * b_scale
            logits.append(jnp.where(pos >= w * B_DIL, acc, NEG) if w else acc)
        mx = functools.reduce(jnp.maximum, logits)
        ex = [jnp.exp(l - mx) for l in logits]
        inv = 1.0 / functools.reduce(jnp.add, ex)
        return jnp.concatenate([
            inv * functools.reduce(jnp.add, [ex[w] * qkv_v[2 * DT + t, rows[w], :] for w in range(B_WIN)])
            for t in range(DT)], axis=1)

    task = functools.partial

    def b_block(blk, side):
        def one(r, c):
            top = pl.multiple_of(blk * B_BLK + r, B_MM)
            qkv_v[c, pl.ds(top + B_PAD, B_MM), :] = b_project(x_v[pl.ds(top, B_MM), :], c)

        _interleave([task(one, r, c) for r in range(0, B_BLK, B_MM) for c in range(3 * DT)], side)

    def slab(tile):
        return pl.ds(pl.multiple_of(tile * LANES, LANES), LANES)

    def a_queries(i, side):
        def one(r, tile):
            qpre_v[tile, r:r + B_MM, :] = _nt(xpre_v[r:r + B_MM, :], stage[0, slab(tile), :])

        _interleave([task(one, r, i * q_tiles + k) for k in range(q_tiles)
                     for r in range(0, n_seg * Q_PRE, B_MM)], side)

    def retile(m, tile, t, src=None):
        src_m, src_tile = src or (m, tile)
        w = stage[src_m, slab(src_tile), t * LANES:(t + 1) * LANES]
        if m < 3:
            w_v[m, tile, t * LANES // 2:(t + 1) * LANES // 2, :] = _pack(w.T)
        else:
            wo_v[t, pl.ds(pl.multiple_of(tile * (LANES // 2), LANES // 2), LANES // 2), :] = _pack(w)

    def retile_q(i):
        return [task(retile, 0, i * q_tiles + k, t) for k in range(q_tiles) for t in range(DT)]

    def phase0(i, carry):
        @pl.when(i > 0)
        def _():
            cp_w(0, i + 1).start()

        @pl.when(i + 2 < n_blk)
        def _():
            cp_w(2, i).start()
            cp_w(3, i).start()

        @pl.when(i + 3 < n_blk)
        def _():
            cp_w(1, i + 1).start()

        @pl.when(i + 3 == n_blk)
        def _():
            cp_w(1, n_blk - 2, True).start()

        @pl.when(i + 2 == n_blk)
        def _():
            for cp in cp_late + [cp_w(m, n_blk - 2, True) for m in (2, 3)]:
                cp.start()

        cp_w(0, i).wait()

        @pl.when(i > 0)
        def _():
            for m in range(1, 4):
                cp_w(m, i - 1).wait()

        side = retile_q(i)
        later = jnp.minimum(i, 1)
        for k in range(r_tiles):
            tile = (i - later) * r_tiles + k
            side += [task(retile, m, tile, t, (m * later, tile * later)) for t in range(DT) for m in range(1, 4)]
        n = len(side) * SPLIT // 100
        a_queries(i, side[:n])
        b_block(i + 1, side[n:])

    prep = [task(fn, m * DT + t) for m in range(3) for fn in (b_transpose, b_gather) for t in range(DT)]
    for fn in prep[:2 * DT]:
        fn()
    cp_w(0, 1).start()
    b_block(0, prep[2 * DT:] + [lambda: None] * (8 * DT))
    for c in range(DT, 3 * DT):
        qkv_v[c, 0:B_PAD, :] = jnp.broadcast_to(qkv_v[c, B_PAD:B_PAD + 1, :], (B_PAD, LANES))
    cp_w(1, 0).start()
    cp_x1.wait()

    for s in range(0, n_seg, 2):
        tails = [x_v[e - 2 * Q_PRE:e, :].astype(F32)[Q_PRE:] for e in ((s + 1) * seg, (s + 2) * seg)]
        xpre_v[s * Q_PRE:(s + 2) * Q_PRE, :] = jnp.concatenate(tails, axis=0).astype(BF16)

    jax.lax.fori_loop(0, n_blk - 1, phase0, None)
    cp_w(0, n_blk - 1).wait()
    for cp in cp_late + [cp_w(m, n_blk - 2, True) for m in (1, 2, 3)]:
        cp.wait()

    def b_out_weights(t):
        perm_v[t, 0:D, :] = bwo_raw[:, t * LANES:(t + 1) * LANES].astype(F32)
        bwo_v[t] = _pack(interleaved(t, 0, range(db)))

    a_queries(n_blk - 1, retile_q(n_blk - 1) + [
        task(retile, m, (n_blk - 2) * r_tiles + k, t)
        for k in range(r_last) for t in range(DT) for m in range(1, 4)] + [task(b_out_weights, t) for t in range(DT)])

    h_v[0:M, :] = mem0_v[...].astype(F32)
    gate = gate_v[...].astype(F32).reshape(1, D)
    a_scale = dh ** -0.5
    split = dh - LANES

    def segment(s):
        base = pl.multiple_of(s * seg, seg)
        xs = x_v[pl.ds(base, seg), :].astype(F32)
        h_v[M:L, :] = xs
        pre = pl.ds(pl.multiple_of(s * Q_PRE, Q_PRE), Q_PRE)

        lo = _iota((L, LANES), 1) < split
        zero = jnp.zeros((L, LANES), F32)
        row, col = _iota((L, 2 * L), 0), _iota((L, 2 * L), 1)
        even = col < L
        visible = (row < M) | (row >= jnp.where(even, col, col - L))

        def project(m, j):
            return [_nn(h_v[...], _unpack(w_v[m, j * PT + t])) for t in range(PT)]

        def two_heads(y):
            top = jnp.concatenate([y[0], jnp.where(lo, y[1], 0.0), zero], axis=1)
            bot = jnp.concatenate([zero, jnp.where(lo, 0.0, y[1]), y[2]], axis=1)
            return jnp.concatenate([top, bot], axis=0).astype(BF16)

        def softmax(sc):
            sc = jnp.where(visible, sc * a_scale, NEG)
            m0 = jnp.max(jnp.where(even, sc, -jnp.inf), axis=1, keepdims=True)
            m1 = jnp.max(jnp.where(even, -jnp.inf, sc), axis=1, keepdims=True)
            e = jnp.exp(sc - jnp.where(even, m0, m1))
            s0 = jnp.sum(jnp.where(even, e, 0.0), axis=1, keepdims=True)
            s1 = jnp.sum(jnp.where(even, 0.0, e), axis=1, keepdims=True)
            return e / jnp.where(even, s0, s1)

        q, k, v, p, o, b, acc = {}, {}, {}, {}, {}, {}, [None] * DT
        for op, j in _schedule(n_pair, DT):
            if op == "K":
                k[j] = two_heads(project(1, j))
            elif op == "Q":
                q[j] = jnp.concatenate([
                    jnp.concatenate([_nn(h_v[0:L - Q_PRE, :], _unpack(w_v[0, c])), qpre_v[c, pre, :]], axis=0)
                    for c in range(j * PT, (j + 1) * PT)], axis=1)
            elif op == "V":
                v[j] = two_heads(project(2, j))
            elif op == "S":
                p[j] = softmax(_nt(q.pop(j), k.pop(j)))
            elif op == "P":
                o[j] = _nn(p.pop(j), v.pop(j))
            elif op == "O":
                oj = o.pop(j)
                for t in range(DT):
                    y = _nn(oj, _unpack(wo_v[t, j * dh:(j + 1) * dh, :]))
                    acc[t] = y if acc[t] is None else acc[t] + y
            elif op == "W":
                ob = window_attention(base)
            else:
                b[j] = _nn(ob, _unpack(bwo_v[j]))

        g = jax.nn.sigmoid(jnp.sum(xs * gate, axis=1, keepdims=True))
        for t in range(DT):
            lanes = slice(t * LANES, (t + 1) * LANES)
            h_v[0:M, lanes] = acc[t][0:M]
            out_v[pl.ds(base, seg), lanes] = (g * acc[t][M:L] + (1.0 - g) * b[t]).astype(out_v.dtype)

    def step(i, carry):
        for u in range(UNROLL):
            segment(i * UNROLL + u)
        rows = pl.ds(pl.multiple_of(i * (UNROLL * seg), UNROLL * seg), UNROLL * seg)
        pltpu.make_async_copy(out_v.at[rows], out_hbm.at[rows], sem_out).start()
        return carry

    jax.lax.fori_loop(0, n_seg // UNROLL, step, 0)
    pltpu.make_async_copy(out_v, out_hbm, sem_out).wait()


@functools.partial(jax.jit, static_argnames=("A_seg_len",))
def pallas_gated_mix__memory_aug_recurrent_mem_tr__sliding_local_dilated__prompt_kernel(
    A_x: jax.Array,
    A_mem0: jax.Array,
    A_Wq: jax.Array,
    A_Wk: jax.Array,
    A_Wv: jax.Array,
    A_Wo: jax.Array,
    A_seg_len: int,
    B_x: jax.Array,
    B_wqkv: jax.Array,
    B_wo: jax.Array,
    gate_w: jax.Array,
):
    del B_x
    batch, S, D = A_x.shape
    _, H, dh = A_Wq.shape
    M = A_mem0.shape[1]
    E = H * dh
    seg = int(A_seg_len)
    assert batch == 1 and D % LANES == 0 and 2 * dh == 3 * LANES and H % 2 == 0
    assert S % B_BLK == 0 and S % seg == 0 and E % (S // B_BLK * LANES) == 0

    def w_t(w):
        return jnp.transpose(w, (1, 2, 0)).reshape(E, D)

    hbm = pl.BlockSpec(memory_space=pl.ANY)
    DT = D // LANES
    out = pl.pallas_call(
        functools.partial(_kernel, seg=seg, dh=dh),
        out_shape=jax.ShapeDtypeStruct((S, D), A_x.dtype),
        in_specs=[hbm] * 9,
        out_specs=hbm,
        scratch_shapes=[
            pltpu.VMEM((S, D), BF16),
            pltpu.VMEM((4, E, D), BF16),
            pltpu.VMEM((3, E // LANES, D // 2, LANES), U32),
            pltpu.VMEM((DT, E // 2, LANES), U32),
            pltpu.VMEM((D, 3 * D), BF16),
            pltpu.VMEM((D, D), BF16),
            pltpu.VMEM((3 * DT, DT, LANES // 2, LANES), U32),
            pltpu.VMEM((DT, D // 2, LANES), U32),
            pltpu.VMEM((DT, 3 * D, LANES), F32),
            pltpu.VMEM((3 * DT, B_PAD + S, LANES), F32),
            pltpu.VMEM((S // seg * Q_PRE, D), BF16),
            pltpu.VMEM((E // LANES, S // seg * Q_PRE, LANES), F32),
            pltpu.VMEM((M + seg, D), F32),
            pltpu.VMEM((S, D), A_x.dtype),
            pltpu.VMEM((M, D), BF16),
            pltpu.VMEM((D,), BF16),
            pltpu.SemaphoreType.DMA((6,)),
            pltpu.SemaphoreType.DMA((4, S // B_BLK)),
            pltpu.SemaphoreType.DMA(()),
        ],
        compiler_params=pltpu.CompilerParams(vmem_limit_bytes=120 * 1024 * 1024),
    )(
        A_x.reshape(S, D), A_mem0.reshape(M, D), w_t(A_Wq), w_t(A_Wk), w_t(A_Wv),
        A_Wo.reshape(E, D), B_wqkv, B_wo, gate_w,
    )
    return out.reshape(batch, S, D)
```

```python
import functools

import jax
import jax.numpy as jnp
import jax.experimental.pallas as pl
import jax.experimental.pallas.tpu as pltpu

F32 = jnp.float32
BF16 = jnp.bfloat16
U32 = jnp.uint32
LANES, SUBLANES = 128, 8
NEG = -1000000000.0

B_HEADS, B_WIN, B_DIL = 32, 8, 2
B_PAD = 16
B_BLK = 256
B_MM = 128
Q_PRE = SUBLANES
UNROLL = 4
STAGES = (("K", 0), ("Q", 0), ("P", 2), ("V", 0), ("S", 0), ("O", 3))


def _nn(a, b):
    return jax.lax.dot_general(a, b, (((1,), (0,)), ((), ())), preferred_element_type=F32)


def _nt(a, b):
    return jax.lax.dot_general(a, b, (((1,), (1,)), ((), ())), preferred_element_type=F32)


def _pack(w):
    return pltpu.bitcast(w, U32)


def _unpack(w):
    return pltpu.bitcast(w, BF16)


def _iota(shape, dim):
    return jax.lax.broadcasted_iota(jnp.int32, shape, dim)


def _interleave(main, side):
    for n, fn in enumerate(main):
        fn()
        for extra in side[n * len(side) // len(main):(n + 1) * len(side) // len(main)]:
            extra()


def _schedule(n_pair, n_tile, early):
    ops = []
    for j in range(n_pair + max(lag for _, lag in STAGES)):
        ops += [(op, j - lag) for op, lag in STAGES if 0 <= j - lag < n_pair]
    ops.insert(len(ops) // 3, ("W", 0))
    at = ops.index(("P", n_pair - 1))
    fill = [("B", t) for t in range(n_tile)]
    return ops[:at] + fill[:early] + ops[at:] + fill[early:]


def _kernel(x_hbm, mem0_hbm, wq_hbm, wk_hbm, wv_hbm, wo_hbm, bqkv_hbm, bwo_hbm, gate_hbm,
            out_hbm,
            x_v, stage, w_v, wo_v, bqkv_raw, bwo_raw, bqkv_v, bwo_v, perm_v, qkv_v,
            xpre_v, qpre_v, h_v, out_v, mem0_v, gate_v, sem_in, sem_w, sem_out, *, seg, dh):
    S, D = x_v.shape
    M = mem0_v.shape[0]
    L = M + seg
    E = stage.shape[1]
    DT = D // LANES
    PT = 2 * dh // LANES
    n_pair = E // (2 * dh)
    n_seg = S // seg
    n_blk = S // B_BLK
    q_tiles = E // LANES // n_blk
    r_tiles = pl.cdiv(E // LANES, n_blk - 1)
    r_last = E // LANES - (n_blk - 2) * r_tiles
    w_hbm = (wq_hbm, wk_hbm, wv_hbm, wo_hbm)

    cp_bqkv = pltpu.make_async_copy(bqkv_hbm, bqkv_raw, sem_in.at[0])
    head, tail = pl.ds(0, B_BLK), pl.ds(B_BLK, S - B_BLK)
    cp_x0 = pltpu.make_async_copy(x_hbm.at[head], x_v.at[head], sem_in.at[1])
    cp_x1 = pltpu.make_async_copy(x_hbm.at[tail], x_v.at[tail], sem_in.at[2])
    cp_late = [pltpu.make_async_copy(src, dst, sem_in.at[3 + n])
               for n, (src, dst) in enumerate(((bwo_hbm, bwo_raw), (mem0_hbm, mem0_v), (gate_hbm, gate_v)))]

    def cp_w(m, c, last=False):
        n = (r_tiles if m else q_tiles) * LANES
        rows = pl.ds(c * n, r_last * LANES if last else n)
        return pltpu.make_async_copy(w_hbm[m].at[rows], stage.at[m, rows], sem_w.at[m, c])

    cp_bqkv.start()
    cp_x0.start()
    cp_x0.wait()
    cp_bqkv.wait()
    cp_x1.start()
    cp_w(0, 0).start()

    db = D // B_HEADS

    def interleaved(t, first, ds):
        return jnp.concatenate(
            [perm_v[t, pl.ds(first + d, B_HEADS, stride=db), :] for d in ds], axis=0).astype(BF16)

    def b_transpose(c):
        wt = bqkv_raw[:, c * LANES:(c + 1) * LANES].T.astype(F32)
        for t in range(DT):
            perm_v[t, c * LANES:(c + 1) * LANES, :] = wt[:, t * LANES:(t + 1) * LANES]

    def b_gather(c):
        per_tile = LANES // B_HEADS
        ds = range(c % DT * per_tile, (c % DT + 1) * per_tile)
        for t in range(DT):
            bqkv_v[c, t] = _pack(interleaved(t, c // DT * D, ds))

    def b_project(xb, c):
        return _nt(xb, jnp.concatenate([_unpack(bqkv_v[c, t]) for t in range(DT)], axis=1))

    b_scale = db ** -0.5

    def window_attention(base):
        q = [qkv_v[t, pl.ds(base + B_PAD, seg), :] for t in range(DT)]
        pos = base + _iota((seg, LANES), 0)
        rows = [pl.ds(base + (B_PAD - w * B_DIL), seg) for w in range(B_WIN)]
        logits = []
        for w in range(B_WIN):
            acc = functools.reduce(jnp.add, [q[t] * qkv_v[DT + t, rows[w], :] for t in range(DT)])
            shift = LANES // 2
            while shift >= B_HEADS:
                acc = acc + pltpu.roll(acc, shift, 1)
                shift //= 2
            acc = acc * b_scale
            logits.append(jnp.where(pos >= w * B_DIL, acc, NEG) if w else acc)
        mx = functools.reduce(jnp.maximum, logits)
        ex = [jnp.exp(l - mx) for l in logits]
        inv = 1.0 / functools.reduce(jnp.add, ex)
        return jnp.concatenate([
            inv * functools.reduce(jnp.add, [ex[w] * qkv_v[2 * DT + t, rows[w], :] for w in range(B_WIN)])
            for t in range(DT)], axis=1)

    task = functools.partial

    def b_block(blk, side):
        def one(r, c):
            top = pl.multiple_of(blk * B_BLK + r, B_MM)
            qkv_v[c, pl.ds(top + B_PAD, B_MM), :] = b_project(x_v[pl.ds(top, B_MM), :], c)

        _interleave([task(one, r, c) for r in range(0, B_BLK, B_MM) for c in range(3 * DT)], side)

    def slab(tile):
        return pl.ds(pl.multiple_of(tile * LANES, LANES), LANES)

    def a_queries(i, side):
        def one(r, tile):
            qpre_v[tile, r:r + B_MM, :] = _nt(xpre_v[r:r + B_MM, :], stage[0, slab(tile), :])

        _interleave([task(one, r, i * q_tiles + k) for k in range(q_tiles)
                     for r in range(0, n_seg * Q_PRE, B_MM)], side)

    def retile(m, tile, t, src=None):
        src_m, src_tile = src or (m, tile)
        w = stage[src_m, slab(src_tile), t * LANES:(t + 1) * LANES]
        if m < 3:
            w_v[m, tile, t * LANES // 2:(t + 1) * LANES // 2, :] = _pack(w.T)
        else:
            wo_v[t, pl.ds(pl.multiple_of(tile * (LANES // 2), LANES // 2), LANES // 2), :] = _pack(w)

    def retile_q(i):
        return [task(retile, 0, i * q_tiles + k, t) for k in range(q_tiles) for t in range(DT)]

    def phase0(i, carry):
        @pl.when(i > 0)
        def _():
            cp_w(0, i + 1).start()

        @pl.when(i + 2 < n_blk)
        def _():
            cp_w(2, i).start()
            cp_w(3, i).start()

        @pl.when(i + 3 < n_blk)
        def _():
            cp_w(1, i + 1).start()

        @pl.when(i + 3 == n_blk)
        def _():
            cp_w(1, n_blk - 2, True).start()

        @pl.when(i + 2 == n_blk)
        def _():
            for cp in cp_late + [cp_w(m, n_blk - 2, True) for m in (2, 3)]:
                cp.start()

        cp_w(0, i).wait()

        @pl.when(i > 0)
        def _():
            for m in range(1, 4):
                cp_w(m, i - 1).wait()

        side = retile_q(i)
        later = jnp.minimum(i, 1)
        for k in range(r_tiles):
            tile = (i - later) * r_tiles + k
            side += [task(retile, m, tile, t, (m * later, tile * later)) for t in range(DT) for m in range(1, 4)]
        n = len(side) // 2
        a_queries(i, side[:n])
        b_block(i + 1, side[n:])

    prep = [task(fn, m * DT + t) for m in range(3) for fn in (b_transpose, b_gather) for t in range(DT)]
    for fn in prep[:2 * DT]:
        fn()
    cp_w(0, 1).start()
    b_block(0, prep[2 * DT:] + [lambda: None] * (8 * DT))
    for c in range(DT, 3 * DT):
        qkv_v[c, 0:B_PAD, :] = jnp.broadcast_to(qkv_v[c, B_PAD:B_PAD + 1, :], (B_PAD, LANES))
    cp_w(1, 0).start()
    cp_x1.wait()

    for s in range(0, n_seg, 2):
        tails = [x_v[e - 2 * Q_PRE:e, :].astype(F32)[Q_PRE:] for e in ((s + 1) * seg, (s + 2) * seg)]
        xpre_v[s * Q_PRE:(s + 2) * Q_PRE, :] = jnp.concatenate(tails, axis=0).astype(BF16)

    jax.lax.fori_loop(0, n_blk - 1, phase0, None)
    cp_w(0, n_blk - 1).wait()
    for cp in cp_late + [cp_w(m, n_blk - 2, True) for m in (1, 2, 3)]:
        cp.wait()

    def b_out_weights(t):
        perm_v[t, 0:D, :] = bwo_raw[:, t * LANES:(t + 1) * LANES].astype(F32)
        bwo_v[t] = _pack(interleaved(t, 0, range(db)))

    a_queries(n_blk - 1, retile_q(n_blk - 1) + [
        task(retile, m, (n_blk - 2) * r_tiles + k, t)
        for k in range(r_last) for t in range(DT) for m in range(1, 4)] + [task(b_out_weights, t) for t in range(DT)])

    h_v[0:M, :] = mem0_v[...].astype(F32)
    gate = gate_v[...].astype(F32).reshape(1, D)
    a_scale = dh ** -0.5
    split = dh - LANES

    def segment(s, last):
        base = pl.multiple_of(s * seg, seg)
        xs = x_v[pl.ds(base, seg), :].astype(F32)
        h_v[M:L, :] = xs
        pre = pl.ds(pl.multiple_of(s * Q_PRE, Q_PRE), Q_PRE)

        lo = _iota((L, LANES), 1) < split
        zero = jnp.zeros((L, LANES), F32)
        row, col = _iota((L, 2 * L), 0), _iota((L, 2 * L), 1)
        even = col < L
        visible = (row < M) | (row >= jnp.where(even, col, col - L))

        def project(m, j):
            return [_nn(h_v[...], _unpack(w_v[m, j * PT + t])) for t in range(PT)]

        def two_heads(y):
            top = jnp.concatenate([y[0], jnp.where(lo, y[1], 0.0), zero], axis=1)
            bot = jnp.concatenate([zero, jnp.where(lo, 0.0, y[1]), y[2]], axis=1)
            return jnp.concatenate([top, bot], axis=0).astype(BF16)

        def softmax(sc):
            sc = jnp.where(visible, sc * a_scale, NEG)
            m0 = jnp.max(jnp.where(even, sc, -jnp.inf), axis=1, keepdims=True)
            m1 = jnp.max(jnp.where(even, -jnp.inf, sc), axis=1, keepdims=True)
            e = jnp.exp(sc - jnp.where(even, m0, m1))
            s0 = jnp.sum(jnp.where(even, e, 0.0), axis=1, keepdims=True)
            s1 = jnp.sum(jnp.where(even, 0.0, e), axis=1, keepdims=True)
            return e / jnp.where(even, s0, s1)

        q, k, v, p, o, b, acc = {}, {}, {}, {}, {}, {}, [None] * DT
        for op, j in _schedule(n_pair, DT, DT if last else 2):
            if op == "K":
                k[j] = two_heads(project(1, j))
            elif op == "Q":
                q[j] = jnp.concatenate([
                    jnp.concatenate([_nn(h_v[0:L - Q_PRE, :], _unpack(w_v[0, c])), qpre_v[c, pre, :]], axis=0)
                    for c in range(j * PT, (j + 1) * PT)], axis=1)
            elif op == "V":
                v[j] = two_heads(project(2, j))
            elif op == "S":
                p[j] = softmax(_nt(q.pop(j), k.pop(j)))
            elif op == "P":
                o[j] = _nn(p.pop(j), v.pop(j))
            elif op == "O":
                oj = o.pop(j)
                for t in range(DT):
                    y = _nn(oj, _unpack(wo_v[t, j * dh:(j + 1) * dh, :]))
                    acc[t] = y if acc[t] is None else acc[t] + y
            elif op == "W":
                ob = window_attention(base)
            else:
                b[j] = _nn(ob, _unpack(bwo_v[j]))

        g = jax.nn.sigmoid(jnp.sum(xs * gate, axis=1, keepdims=True))
        for t in range(DT):
            lanes = slice(t * LANES, (t + 1) * LANES)
            h_v[0:M, lanes] = acc[t][0:M]
            out_v[pl.ds(base, seg), lanes] = (g * acc[t][M:L] + (1.0 - g) * b[t]).astype(out_v.dtype)

    def step(i, carry):
        for u in range(UNROLL):
            segment(i * UNROLL + u, u == UNROLL - 1)
        rows = pl.ds(pl.multiple_of(i * (UNROLL * seg), UNROLL * seg), UNROLL * seg)
        pltpu.make_async_copy(out_v.at[rows], out_hbm.at[rows], sem_out).start()
        return carry

    jax.lax.fori_loop(0, n_seg // UNROLL, step, 0)
    pltpu.make_async_copy(out_v, out_hbm, sem_out).wait()


@functools.partial(jax.jit, static_argnames=("A_seg_len",))
def pallas_gated_mix__memory_aug_recurrent_mem_tr__sliding_local_dilated__prompt_kernel(
    A_x: jax.Array,
    A_mem0: jax.Array,
    A_Wq: jax.Array,
    A_Wk: jax.Array,
    A_Wv: jax.Array,
    A_Wo: jax.Array,
    A_seg_len: int,
    B_x: jax.Array,
    B_wqkv: jax.Array,
    B_wo: jax.Array,
    gate_w: jax.Array,
):
    del B_x
    batch, S, D = A_x.shape
    _, H, dh = A_Wq.shape
    M = A_mem0.shape[1]
    E = H * dh
    seg = int(A_seg_len)
    assert batch == 1 and D % LANES == 0 and 2 * dh == 3 * LANES and H % 2 == 0
    assert M % SUBLANES == 0 and seg % (2 * Q_PRE) == 0 and S % (UNROLL * seg) == 0
    assert S % B_BLK == 0 and S % seg == 0 and E % (S // B_BLK * LANES) == 0

    def w_t(w):
        return jnp.transpose(w, (1, 2, 0)).reshape(E, D)

    hbm = pl.BlockSpec(memory_space=pl.ANY)
    DT = D // LANES
    out = pl.pallas_call(
        functools.partial(_kernel, seg=seg, dh=dh),
        out_shape=jax.ShapeDtypeStruct((S, D), A_x.dtype),
        in_specs=[hbm] * 9,
        out_specs=hbm,
        scratch_shapes=[
            pltpu.VMEM((S, D), BF16),
            pltpu.VMEM((4, E, D), BF16),
            pltpu.VMEM((3, E // LANES, D // 2, LANES), U32),
            pltpu.VMEM((DT, E // 2, LANES), U32),
            pltpu.VMEM((D, 3 * D), BF16),
            pltpu.VMEM((D, D), BF16),
            pltpu.VMEM((3 * DT, DT, LANES // 2, LANES), U32),
            pltpu.VMEM((DT, D // 2, LANES), U32),
            pltpu.VMEM((DT, 3 * D + 32, LANES), F32),
            pltpu.VMEM((3 * DT, B_PAD + S, LANES), F32),
            pltpu.VMEM((S // seg * Q_PRE, D), BF16),
            pltpu.VMEM((E // LANES, S // seg * Q_PRE, LANES), F32),
            pltpu.VMEM((M + seg, D), F32),
            pltpu.VMEM((S, D), A_x.dtype),
            pltpu.VMEM((M, D), BF16),
            pltpu.VMEM((D,), BF16),
            pltpu.SemaphoreType.DMA((6,)),
            pltpu.SemaphoreType.DMA((4, S // B_BLK)),
            pltpu.SemaphoreType.DMA(()),
        ],
        compiler_params=pltpu.CompilerParams(vmem_limit_bytes=120 * 1024 * 1024),
    )(
        A_x.reshape(S, D), A_mem0.reshape(M, D), w_t(A_Wq), w_t(A_Wk), w_t(A_Wv),
        A_Wo.reshape(E, D), B_wqkv, B_wo, gate_w,
    )
    return out.reshape(batch, S, D)
```
